```python
import jax
import jax.numpy as jnp

def _softmax(x, axis=-1):
    return jax.nn.softmax(x, axis=axis)
def _gelu(x):
    return jax.nn.gelu(x, approximate=True)
def _silu(x):
    return jax.nn.silu(x)
def _sigmoid(x):
    return jax.nn.sigmoid(x)
def _layernorm(x, axis=-1, eps=1e-5):
    m = jnp.mean(x, axis=axis, keepdims=True)
    v = jnp.var(x, axis=axis, keepdims=True)
    return (x - m) / jnp.sqrt(v + eps)
def _scatter_add(tgt, idx, src, axis=0):
    return tgt.at[idx].add(src)
def _segment_sum(src, seg, n):
    return jax.ops.segment_sum(src, seg, n)
class _Rng:
    def __init__(self, key):
        self._k = key
    def _next(self):
        self._k, sub = jax.random.split(self._k)
        return sub
    def normal(self, shape):
        return jax.random.normal(self._next(), shape, dtype=jnp.bfloat16)
    def randint(self, lo, hi, shape):
        return jax.random.randint(self._next(), shape, lo, hi, dtype=jnp.int32)
    def uniform(self, shape, lo=0.0, hi=1.0):
        return jax.random.uniform(self._next(), shape, jnp.bfloat16, lo, hi)
    def permutation(self, n):
        return jax.random.permutation(self._next(), n)


kernel_name = 'gated_mix__compressed_kv_cla__gqa_block_cached__decode'

def setup_inputs():
    _rng = _Rng(jax.random.key(int.from_bytes(__import__("os").urandom(4), "little")))
    _w = (lambda a: (lambda t: t.astype(jnp.bfloat16) if jnp.issubdtype(t.dtype, jnp.floating) else t)(jnp.asarray(a)))
    def _A_setup():
        B, H, Sq, Sk, D, M = 1, 32, 1, 4096, 128, 640
        Dc = 4 * D
        return {
            "x": _w((lambda *s: _rng.normal(s) * 0.05)(B, Sq, M)),
            "c_kv": _w((lambda *s: _rng.normal(s) * 0.05)(B, Sk, Dc)),
            "w_q": _w((lambda *s: _rng.normal(s) * 0.05)(M, H, D) * (M ** -0.5)),
            "w_uk": _w((lambda *s: _rng.normal(s) * 0.05)(Dc, H, D) * (Dc ** -0.5)),
            "w_uv": _w((lambda *s: _rng.normal(s) * 0.05)(Dc, H, D) * (Dc ** -0.5)),
            "w_o": _w((lambda *s: _rng.normal(s) * 0.05)(H, D, M) * ((H * D) ** -0.5)),
        }
    _A_in = _A_setup()

    def _B_setup():
        B, Sq, D = 1, 1, 640
        Hq, Hkv, Sk, Dh = 32, 32, 4096, 128
        assert Hq % Hkv == 0, (Hq, Hkv)
        return {
            "x": _w((lambda *s: _rng.normal(s) * 0.05)(B, Sq, D)),
            "k_cache": _w((lambda *s: _rng.normal(s) * 0.05)(B, Hkv, Sk, Dh)),
            "v_cache": _w((lambda *s: _rng.normal(s) * 0.05)(B, Hkv, Sk, Dh)),
            "wq": _w((lambda *s: _rng.normal(s) * 0.05)(D, Hq * Dh) * (D ** -0.5)),
            "wo": _w((lambda *s: _rng.normal(s) * 0.05)(Hq * Dh, D) * ((Hq * Dh) ** -0.5)),
        }
    _B_in = _B_setup()

    return {
        "A_x": _A_in["x"],
        "A_c_kv": _A_in["c_kv"],
        "A_w_q": _A_in["w_q"],
        "A_w_uk": _A_in["w_uk"],
        "A_w_uv": _A_in["w_uv"],
        "A_w_o": _A_in["w_o"],
        "B_x": _B_in["x"],
        "B_k_cache": _B_in["k_cache"],
        "B_v_cache": _B_in["v_cache"],
        "B_wq": _B_in["wq"],
        "B_wo": _B_in["wo"],
        "gate_w": _w((lambda *s: _rng.normal(s) * 0.05)(640)),
    }

def reference(A_x, A_c_kv, A_w_q, A_w_uk, A_w_uv, A_w_o, B_x, B_k_cache, B_v_cache, B_wq, B_wo, gate_w):
    def _A_ref(x, c_kv, w_q, w_uk, w_uv, w_o):
        B, Sq, M = x.shape[0], x.shape[1], x.shape[2]
        Sk = c_kv.shape[1]
        H, D = w_q.shape[1], w_q.shape[2]
        q = jnp.einsum("bqm,mhd->bhqd", x, w_q)
        k = jnp.einsum("bkc,chd->bhkd", c_kv, w_uk)
        v = jnp.einsum("bkc,chd->bhkd", c_kv, w_uv)
        scores = jnp.einsum("bhqd,bhkd->bhqk", q, k) * (D ** -0.5)
        off = Sk - Sq
        qi = jnp.arange(Sq)[:, None]
        kj = jnp.arange(Sk)[None, :]
        cmask = kj <= (qi + off)
        scores = jnp.where(cmask[None, None], scores, -1e9)
        p = _softmax(scores, axis=-1)
        ctx = jnp.einsum("bhqk,bhkd->bhqd", p, v)
        return jnp.einsum("bhqd,hdm->bqm", ctx, w_o)

    def _B_ref(x, k_cache, v_cache, wq, wo):
        B, Sq, D = x.shape
        Hq, Dh = 32, 128
        Hkv = k_cache.shape[1]
        rep = Hq // Hkv
        q = (lambda x, *d: x.transpose(*d))((x @ wq).reshape(B, Sq, Hq, Dh), 0, 2, 1, 3)
        k = jnp.repeat(k_cache, rep, axis=1)
        v = jnp.repeat(v_cache, rep, axis=1)
        scores = jnp.einsum("bhqd,bhkd->bhqk", q, k) * (Dh ** -0.5)
        p = _softmax(scores, axis=-1)
        o = jnp.einsum("bhqk,bhkd->bhqd", p, v)
        return (lambda x, *d: x.transpose(*d))(o, 0, 2, 1, 3).reshape(B, Sq, Hq * Dh) @ wo

    x = A_x
    g = _sigmoid((x * gate_w).sum(-1, keepdims=True))
    a = _A_ref(x, A_c_kv, A_w_q, A_w_uk, A_w_uv, A_w_o)
    b = _B_ref(x, B_k_cache, B_v_cache, B_wq, B_wo)
    return g * a + (1 - g) * b
```

```python
import jax
import jax.numpy as jnp
from jax import lax
import jax.experimental.pallas as pl
import jax.experimental.pallas.tpu as pltpu

_NT = (((1,), (1,)), ((), ()))
_F32 = jnp.float32
_BF16 = jnp.bfloat16

NBUF = 3
WO_CHUNKS = (1024, 1024, 1024, 512, 256, 128, 128)


def _dot(a, b):
    return jnp.dot(a, b, preferred_element_type=_F32)


def _dot_nt(a, b):
    return lax.dot_general(a, b, _NT, preferred_element_type=_F32)


@jax.jit
def pallas_gated_mix__compressed_kv_cla__gqa_block_cached__decode_kernel(
    A_x: jax.Array,
    A_c_kv: jax.Array,
    A_w_q: jax.Array,
    A_w_uk: jax.Array,
    A_w_uv: jax.Array,
    A_w_o: jax.Array,
    B_x: jax.Array,
    B_k_cache: jax.Array,
    B_v_cache: jax.Array,
    B_wq: jax.Array,
    B_wo: jax.Array,
    gate_w: jax.Array,
):
    B, Sq, M = A_x.shape
    _, Sk, Dc = A_c_kv.shape
    _, H, D = A_w_q.shape
    assert B == 1 and Sq == 1 and D == 128 and H == 32
    assert B_k_cache.shape == (1, H, Sk, D) and B_v_cache.shape == (1, H, Sk, D)
    assert sum(WO_CHUNKS) == H * D
    HD = H * D
    scale = float(D) ** -0.5
    NXC = M // 128
    NCB = Dc // 128

    w_q2 = A_w_q.reshape(M * H, D)
    w_uk2 = A_w_uk.reshape(Dc * H, D)
    w_uv2 = A_w_uv.reshape(Dc * H, D)
    w_o2 = A_w_o.reshape(HD, M)

    def kernel(x_hbm, gw_hbm, wqb_hbm, k_hbm, v_hbm, wqa_hbm, wuk_hbm, ckv_hbm,
               wuv_hbm, woa_hbm, wob_hbm,
               o_ref,
               x_v, gw_v, wqb_v, kbuf, vbuf, wqa_v, wuk_v, ckv_v, wuv_v, woa_v, wob_v,
               qb_s, ob_s,
               sem_w, sem_k, sem_v, sem_o):
        cp_x = pltpu.make_async_copy(x_hbm, x_v, sem_w.at[0])
        cp_gw = pltpu.make_async_copy(gw_hbm, gw_v, sem_w.at[1])
        cp_wqb = pltpu.make_async_copy(wqb_hbm, wqb_v, sem_w.at[2])
        cp_wqa = pltpu.make_async_copy(wqa_hbm, wqa_v, sem_w.at[3])
        cp_wuk = pltpu.make_async_copy(wuk_hbm, wuk_v, sem_w.at[4])
        cp_ckv = pltpu.make_async_copy(ckv_hbm.at[0], ckv_v, sem_w.at[5])
        cp_wuv = pltpu.make_async_copy(wuv_hbm, wuv_v, sem_w.at[6])
        cp_woa = pltpu.make_async_copy(woa_hbm, woa_v, sem_w.at[7])
        wo_off = [sum(WO_CHUNKS[:i]) for i in range(len(WO_CHUNKS))]
        cp_wob = [
            pltpu.make_async_copy(wob_hbm.at[pl.ds(o, n)], wob_v.at[pl.ds(o, n)], sem_o.at[i])
            for i, (o, n) in enumerate(zip(wo_off, WO_CHUNKS))
        ]

        def cp_k(h, slot):
            return pltpu.make_async_copy(k_hbm.at[0, h], kbuf.at[slot], sem_k.at[slot])

        def cp_v(h, slot):
            return pltpu.make_async_copy(v_hbm.at[0, h], vbuf.at[slot], sem_v.at[slot])

        cp_x.start()
        cp_gw.start()
        cp_wqb.start()
        for h in range(NBUF):
            cp_k(h, h).start()
            cp_v(h, h).start()

        e_row = lax.broadcasted_iota(jnp.int32, (128, HD), 0)
        e_col = lax.broadcasted_iota(jnp.int32, (128, HD), 1)
        e0 = jnp.where(e_row == (e_col >> 5), 1.0, 0.0).astype(_BF16)
        d_row = lax.broadcasted_iota(jnp.int32, (H, HD), 0)
        d_col = lax.broadcasted_iota(jnp.int32, (H, HD), 1)
        diag = (d_col & (H - 1)) == d_row

        cp_x.wait()
        cp_gw.wait()
        x = x_v[0].astype(_F32)
        gw = gw_v[...].astype(_F32).reshape(1, M)
        g = jax.nn.sigmoid(jnp.sum(x * gw, axis=-1, keepdims=True))
        x8 = jnp.broadcast_to(x, (8, M)).astype(_BF16)

        cp_wqb.wait()
        qb = _dot(x8, wqb_v[...]) * scale
        for h in range(H):
            qb_s[h] = qb[:, h * D:(h + 1) * D]

        def attend(h, slot):
            cp_k(h, slot).wait()
            q = qb_s[h].astype(_BF16)
            s = _dot_nt(q, kbuf[slot])
            m = jnp.max(s, axis=-1, keepdims=True)
            p = jnp.exp(s - m)
            l = jnp.sum(p, axis=-1, keepdims=True)
            cp_v(h, slot).wait()
            o = _dot(p.astype(_BF16), vbuf[slot])
            ob_s[h] = o / l

        def body(h, carry):
            slot = lax.rem(h, NBUF)
            attend(h, slot)
            cp_k(h + NBUF, slot).start()
            cp_v(h + NBUF, slot).start()
            return carry

        lax.fori_loop(0, H - NBUF, body, 0)

        cp_wqa.start()
        cp_wuk.start()
        cp_ckv.start()
        cp_wuv.start()
        cp_woa.start()
        for c in cp_wob:
            c.start()

        for h in range(H - NBUF, H):
            attend(h, h % NBUF)

        x5 = jnp.concatenate(
            [x[:, c * 128:(c + 1) * 128] for c in range(NXC)]
            + [jnp.zeros((8 - NXC, 128), _F32)], axis=0).astype(_BF16)
        xr = _dot(x5, e0)
        cp_wqa.wait()
        qa = jnp.zeros((H, D), _F32)
        for c in range(NXC):
            sc = jnp.where(diag, jnp.broadcast_to(xr[c:c + 1, :], (H, HD)), 0.0).astype(_BF16)
            qa = qa + _dot(sc, wqa_v[pl.ds(c * HD, HD), :])
        qa = (qa * scale).astype(_BF16)

        cp_wuk.wait()
        qabs = []
        for b in range(NCB):
            t = _dot_nt(qa, wuk_v[pl.ds(b * HD, HD), :])
            mb = jnp.where(diag, t, 0.0).astype(_BF16)
            qabs.append(_dot_nt(mb, e0))
        qabs = jnp.concatenate(qabs, axis=1).astype(_BF16)

        cp_ckv.wait()
        ckv = ckv_v[...]
        s = _dot_nt(qabs, ckv)
        m = jnp.max(s, axis=-1, keepdims=True)
        p = jnp.exp(s - m)
        l = jnp.sum(p, axis=-1, keepdims=True)
        cl = (_dot(p.astype(_BF16), ckv) / l).astype(_BF16)

        cp_wuv.wait()
        ctx = jnp.zeros((H, D), _F32)
        for b in range(NCB):
            xb = _dot(cl[:, b * 128:(b + 1) * 128], e0)
            sb = jnp.where(diag, xb, 0.0).astype(_BF16)
            ctx = ctx + _dot(sb, wuv_v[pl.ds(b * HD, HD), :])

        sub = lax.broadcasted_iota(jnp.int32, (8, D), 0)
        ctx_flat = jnp.concatenate(
            [jnp.where(sub == (h % 8), ctx[8 * (h // 8):8 * (h // 8) + 8, :], 0.0) for h in range(H)],
            axis=1).astype(_BF16)
        cp_woa.wait()
        a = jnp.sum(_dot(ctx_flat, woa_v[...]), axis=0, keepdims=True)

        o_flat = jnp.concatenate([ob_s[h] for h in range(H)], axis=1).astype(_BF16)
        one_g = 1.0 - g
        acc = g * a
        for i, (o, n) in enumerate(zip(wo_off, WO_CHUNKS)):
            cp_wob[i].wait()
            part = _dot(o_flat[:, o:o + n], wob_v[pl.ds(o, n), :])
            acc = acc + one_g * part[0:1, :]
        o_ref[0] = acc.astype(o_ref.dtype)

    any_spec = pl.BlockSpec(memory_space=pl.ANY)
    scratch = [
        pltpu.VMEM((1, 1, M), _BF16),
        pltpu.VMEM((M,), _BF16),
        pltpu.VMEM((M, HD), _BF16),
        pltpu.VMEM((NBUF, Sk, D), _BF16),
        pltpu.VMEM((NBUF, Sk, D), _BF16),
        pltpu.VMEM((M * H, D), _BF16),
        pltpu.VMEM((Dc * H, D), _BF16),
        pltpu.VMEM((Sk, Dc), _BF16),
        pltpu.VMEM((Dc * H, D), _BF16),
        pltpu.VMEM((HD, M), _BF16),
        pltpu.VMEM((HD, M), _BF16),
        pltpu.VMEM((H, 8, D), _F32),
        pltpu.VMEM((H, 8, D), _F32),
        pltpu.SemaphoreType.DMA((8,)),
        pltpu.SemaphoreType.DMA((NBUF,)),
        pltpu.SemaphoreType.DMA((NBUF,)),
        pltpu.SemaphoreType.DMA((len(WO_CHUNKS),)),
    ]
    return pl.pallas_call(
        kernel,
        out_shape=jax.ShapeDtypeStruct((B, Sq, M), A_x.dtype),
        in_specs=[any_spec] * 11,
        out_specs=pl.BlockSpec(memory_space=pltpu.VMEM),
        scratch_shapes=scratch,
        compiler_params=pltpu.CompilerParams(vmem_limit_bytes=100 * 1024 * 1024),
    )(A_x, gate_w, B_wq, B_k_cache, B_v_cache, w_q2, w_uk2, A_c_kv, w_uv2, w_o2, B_wo)
```

```python
import jax
import jax.numpy as jnp
from jax import lax
import jax.experimental.pallas as pl
import jax.experimental.pallas.tpu as pltpu

_NT = (((1,), (1,)), ((), ()))
_F32 = jnp.float32
_BF16 = jnp.bfloat16

NBUF = 3
WO_CHUNKS = (1024, 1024, 1024, 512, 256, 128, 128)
NOSEM = False


def _dot(a, b):
    return jnp.dot(a, b, preferred_element_type=_F32)


def _dot_nt(a, b):
    return lax.dot_general(a, b, _NT, preferred_element_type=_F32)


@jax.jit
def pallas_gated_mix__compressed_kv_cla__gqa_block_cached__decode_kernel(
    A_x: jax.Array,
    A_c_kv: jax.Array,
    A_w_q: jax.Array,
    A_w_uk: jax.Array,
    A_w_uv: jax.Array,
    A_w_o: jax.Array,
    B_x: jax.Array,
    B_k_cache: jax.Array,
    B_v_cache: jax.Array,
    B_wq: jax.Array,
    B_wo: jax.Array,
    gate_w: jax.Array,
):
    B, Sq, M = A_x.shape
    _, Sk, Dc = A_c_kv.shape
    _, H, D = A_w_q.shape
    assert B == 1 and Sq == 1 and D == 128 and H == 32
    assert B_k_cache.shape == (1, H, Sk, D) and B_v_cache.shape == (1, H, Sk, D)
    assert sum(WO_CHUNKS) == H * D
    HD = H * D
    scale = float(D) ** -0.5
    NXC = M // 128
    NCB = Dc // 128

    w_q2 = A_w_q.reshape(M * H, D)
    w_uk2 = A_w_uk.reshape(Dc * H, D)
    w_uv2 = A_w_uv.reshape(Dc * H, D)
    w_o2 = A_w_o.reshape(HD, M)

    def kernel(x_hbm, gw_hbm, wqb_hbm, k_hbm, v_hbm, wqa_hbm, wuk_hbm, ckv_hbm,
               wuv_hbm, woa_hbm, wob_hbm,
               o_ref,
               x_v, gw_v, wqb_v, kbuf, vbuf, wqa_v, wuk_v, ckv_v, wuv_v, woa_v, wob_v,
               qb_s, ob_s,
               sem_w, sem_k, sem_v, sem_o):
        cp_x = pltpu.make_async_copy(x_hbm, x_v, sem_w.at[0])
        cp_gw = pltpu.make_async_copy(gw_hbm, gw_v, sem_w.at[1])
        cp_wqb = pltpu.make_async_copy(wqb_hbm, wqb_v, sem_w.at[2])
        cp_wqa = pltpu.make_async_copy(wqa_hbm, wqa_v, sem_w.at[3])
        cp_wuk = pltpu.make_async_copy(wuk_hbm, wuk_v, sem_w.at[4])
        cp_ckv = pltpu.make_async_copy(ckv_hbm.at[0], ckv_v, sem_w.at[5])
        cp_wuv = pltpu.make_async_copy(wuv_hbm, wuv_v, sem_w.at[6])
        cp_woa = pltpu.make_async_copy(woa_hbm, woa_v, sem_w.at[7])
        wo_off = [sum(WO_CHUNKS[:i]) for i in range(len(WO_CHUNKS))]
        cp_wob = [
            pltpu.make_async_copy(wob_hbm.at[pl.ds(o, n)], wob_v.at[pl.ds(o, n)], sem_o.at[i])
            for i, (o, n) in enumerate(zip(wo_off, WO_CHUNKS))
        ]
        tail = [cp_wqa, cp_wuk, cp_ckv, cp_wuv, cp_woa] + cp_wob

        def issue_tail(n=1):
            for _ in range(n):
                if tail:
                    tail.pop(0).start()

        def cp_k(h, slot):
            return pltpu.make_async_copy(k_hbm.at[0, h], kbuf.at[slot], sem_k.at[slot])

        def cp_v(h, slot):
            return pltpu.make_async_copy(v_hbm.at[0, h], vbuf.at[slot], sem_v.at[slot])

        cp_x.start()
        cp_gw.start()
        cp_wqb.start()

        cp_x.wait()
        cp_gw.wait()

        def prime(h, carry):
            cp_k(h, h).start()
            cp_v(h, h).start()
            return carry

        lax.fori_loop(0, NBUF, prime, 0)

        e_row = lax.broadcasted_iota(jnp.int32, (128, HD), 0)
        e_col = lax.broadcasted_iota(jnp.int32, (128, HD), 1)
        e0 = jnp.where(e_row == (e_col >> 5), 1.0, 0.0).astype(_BF16)
        d_row = lax.broadcasted_iota(jnp.int32, (H, HD), 0)
        d_col = lax.broadcasted_iota(jnp.int32, (H, HD), 1)
        diag = (d_col & (H - 1)) == d_row

        x = x_v[0].astype(_F32)
        gw = gw_v[...].astype(_F32).reshape(1, M)
        g = jax.nn.sigmoid(jnp.sum(x * gw, axis=-1, keepdims=True))
        x8 = jnp.broadcast_to(x, (8, M)).astype(_BF16)

        cp_wqb.wait()
        qb = _dot(x8, wqb_v[...]) * scale
        for h in range(H):
            qb_s[h] = qb[:, h * D:(h + 1) * D]

        def attend(h, slot, hook):
            cp_k(h, slot).wait()
            hook()
            q = qb_s[h].astype(_BF16)
            s = _dot_nt(q, kbuf[slot])
            m = jnp.max(s, axis=-1, keepdims=True)
            p = jnp.exp(s - m)
            l = jnp.sum(p, axis=-1, keepdims=True)
            cp_v(h, slot).wait()
            hook()
            o = _dot(p.astype(_BF16), vbuf[slot])
            ob_s[h] = o / l

        def body(h, carry):
            slot = lax.rem(h, NBUF)
            attend(h, slot, lambda: None)
            cp_k(h + NBUF, slot).start()
            cp_v(h + NBUF, slot).start()
            return carry

        lax.fori_loop(0, H - NBUF, body, 0)

        for h in range(H - NBUF, H):
            attend(h, h % NBUF, issue_tail)

        x5 = jnp.concatenate(
            [x[:, c * 128:(c + 1) * 128] for c in range(NXC)]
            + [jnp.zeros((8 - NXC, 128), _F32)], axis=0).astype(_BF16)
        xr = _dot(x5, e0)
        cp_wqa.wait()
        issue_tail()
        qa = jnp.zeros((H, D), _F32)
        for c in range(NXC):
            sc = jnp.where(diag, jnp.broadcast_to(xr[c:c + 1, :], (H, HD)), 0.0).astype(_BF16)
            qa = qa + _dot(sc, wqa_v[pl.ds(c * HD, HD), :])
        qa = (qa * scale).astype(_BF16)

        cp_wuk.wait()
        issue_tail()
        qabs = []
        for b in range(NCB):
            t = _dot_nt(qa, wuk_v[pl.ds(b * HD, HD), :])
            mb = jnp.where(diag, t, 0.0).astype(_BF16)
            qabs.append(_dot_nt(mb, e0))
        qabs = jnp.concatenate(qabs, axis=1).astype(_BF16)

        cp_ckv.wait()
        issue_tail()
        ckv = ckv_v[...]
        s = _dot_nt(qabs, ckv)
        m = jnp.max(s, axis=-1, keepdims=True)
        p = jnp.exp(s - m)
        l = jnp.sum(p, axis=-1, keepdims=True)
        cl = (_dot(p.astype(_BF16), ckv) / l).astype(_BF16)

        cp_wuv.wait()
        issue_tail()
        ctx = jnp.zeros((H, D), _F32)
        for b in range(NCB):
            xb = _dot(cl[:, b * 128:(b + 1) * 128], e0)
            sb = jnp.where(diag, xb, 0.0).astype(_BF16)
            ctx = ctx + _dot(sb, wuv_v[pl.ds(b * HD, HD), :])

        sub = lax.broadcasted_iota(jnp.int32, (8, D), 0)
        ctx_flat = jnp.concatenate(
            [jnp.where(sub == (h % 8), ctx[8 * (h // 8):8 * (h // 8) + 8, :], 0.0) for h in range(H)],
            axis=1).astype(_BF16)
        cp_woa.wait()
        issue_tail()
        a = jnp.sum(_dot(ctx_flat, woa_v[...]), axis=0, keepdims=True)

        o_flat = jnp.concatenate([ob_s[h] for h in range(H)], axis=1).astype(_BF16)
        one_g = 1.0 - g
        acc = g * a
        for i, (o, n) in enumerate(zip(wo_off, WO_CHUNKS)):
            cp_wob[i].wait()
            issue_tail()
            part = _dot(o_flat[:, o:o + n], wob_v[pl.ds(o, n), :])
            acc = acc + one_g * part[0:1, :]
        assert not tail
        o_ref[0] = acc.astype(o_ref.dtype)

    any_spec = pl.BlockSpec(memory_space=pl.ANY)
    scratch = [
        pltpu.VMEM((1, 1, M), _BF16),
        pltpu.VMEM((M,), _BF16),
        pltpu.VMEM((M, HD), _BF16),
        pltpu.VMEM((NBUF, Sk, D), _BF16),
        pltpu.VMEM((NBUF, Sk, D), _BF16),
        pltpu.VMEM((M * H, D), _BF16),
        pltpu.VMEM((Dc * H, D), _BF16),
        pltpu.VMEM((Sk, Dc), _BF16),
        pltpu.VMEM((Dc * H, D), _BF16),
        pltpu.VMEM((HD, M), _BF16),
        pltpu.VMEM((HD, M), _BF16),
        pltpu.VMEM((H, 8, D), _F32),
        pltpu.VMEM((H, 8, D), _F32),
        pltpu.SemaphoreType.DMA((8,)),
        pltpu.SemaphoreType.DMA((NBUF,)),
        pltpu.SemaphoreType.DMA((NBUF,)),
        pltpu.SemaphoreType.DMA((len(WO_CHUNKS),)),
    ]
    return pl.pallas_call(
        kernel,
        out_shape=jax.ShapeDtypeStruct((B, Sq, M), A_x.dtype),
        in_specs=[any_spec] * 11,
        out_specs=pl.BlockSpec(memory_space=pltpu.VMEM),
        scratch_shapes=scratch,
        compiler_params=pltpu.CompilerParams(vmem_limit_bytes=100 * 1024 * 1024, disable_semaphore_checks=NOSEM),
    )(A_x, gate_w, B_wq, B_k_cache, B_v_cache, w_q2, w_uk2, A_c_kv, w_uv2, w_o2, B_wo)
```

```python
import jax
import jax.numpy as jnp
from jax import lax
import jax.experimental.pallas as pl
import jax.experimental.pallas.tpu as pltpu

_NT = (((1,), (1,)), ((), ()))
_F32 = jnp.float32
_BF16 = jnp.bfloat16

UPH = 8
Q0_NUM, Q0_DEN = 1, 4
WLO = 24
WHI = 16
TICK = 4
HB = 8
WO_GROUPS = (8, 8, 8, 4, 2, 1, 1)
NOSEM = True
NOBND = True
PQ0, PQ1 = 0, 1
SKIP_COMPUTE = False
SKIP_A = False
HN = 32


def _dot(a, b):
    return jnp.dot(a, b, preferred_element_type=_F32)


def _dot_nt(a, b):
    return lax.dot_general(a, b, _NT, preferred_element_type=_F32)


class _Unit:
    def __init__(self, hi, lo):
        self.hi, self.lo = hi, lo

    def start_hi(self):
        if self.hi is not None:
            self.hi().start(priority=PQ0)

    def start_lo(self):
        self.lo().start(priority=PQ1)

    def wait_hi(self):
        if self.hi is not None:
            self.hi().wait()

    def wait_lo(self):
        self.lo().wait()


def _row_unit(src, dst, sem, r0, n):
    nh = (n * Q0_NUM // Q0_DEN) // 16 * 16
    until = lambda a, k: pltpu.make_async_copy(src.at[pl.ds(a, k)], dst.at[pl.ds(a, k)], sem)
    if nh == 0:
        return _Unit(None, lambda: until(r0, n))
    return _Unit(lambda: until(r0, nh), lambda: until(r0 + nh, n - nh))


def _col_unit(src, dst, sem, r0, n, ncols):
    ch = (ncols * Q0_NUM // Q0_DEN) // 128 * 128
    until = lambda a, k: pltpu.make_async_copy(
        src.at[pl.ds(r0, n), pl.ds(a, k)], dst.at[pl.ds(r0, n), pl.ds(a, k)], sem)
    if ch == 0:
        return _Unit(None, lambda: until(0, ncols))
    return _Unit(lambda: until(0, ch), lambda: until(ch, ncols - ch))


def _merge(a, b):
    out, i, j = [], 0, 0
    while i < len(a) or j < len(b):
        if j >= len(b) or (i < len(a) and i * len(b) <= j * len(a)):
            out.append(a[i]); i += 1
        else:
            out.append(b[j]); j += 1
    return out


@jax.jit
def pallas_gated_mix__compressed_kv_cla__gqa_block_cached__decode_kernel(
    A_x: jax.Array,
    A_c_kv: jax.Array,
    A_w_q: jax.Array,
    A_w_uk: jax.Array,
    A_w_uv: jax.Array,
    A_w_o: jax.Array,
    B_x: jax.Array,
    B_k_cache: jax.Array,
    B_v_cache: jax.Array,
    B_wq: jax.Array,
    B_wo: jax.Array,
    gate_w: jax.Array,
):
    B, Sq, M = A_x.shape
    _, Sk, Dc = A_c_kv.shape
    _, H, D = A_w_q.shape
    assert B == 1 and Sq == 1 and D == 128 and H == 32
    assert B_k_cache.shape == (1, H, Sk, D) and B_v_cache.shape == (1, H, Sk, D)
    HD = H * D
    scale = float(D) ** -0.5
    NXC = M // 128
    NCB = Dc // 128
    LOOK = -(-WLO // (2 * UPH))
    NBUF = LOOK + 1
    UR = Sk // UPH
    UB = UR * D * 2
    UH = 2 * UPH
    W, W0 = WLO, WHI
    assert W0 <= W
    WO_UR = HD // sum(WO_GROUPS)

    w_q2 = A_w_q.reshape(M * H, D)
    w_uk2 = A_w_uk.reshape(Dc * H, D)
    w_uv2 = A_w_uv.reshape(Dc * H, D)
    w_o2 = A_w_o.reshape(HD, M)

    def kernel(x_hbm, gw_hbm, wqb_hbm, k_hbm, v_hbm, wqa_hbm, wuk_hbm, ckv_hbm,
               wuv_hbm, woa_hbm, wob_hbm,
               o_ref,
               x_v, gw_v, wqb_v, kbuf, vbuf, wqa_v, wuk_v, ckv_v, wuv_v, woa_v, wob_v,
               qb_s, ob_s,
               sem_w, sem_k, sem_v, sem_o):
        cp_x = pltpu.make_async_copy(x_hbm, x_v, sem_w.at[0])
        cp_gw = pltpu.make_async_copy(gw_hbm, gw_v, sem_w.at[1])

        def rows_units(src, dst, sem, nrows, unit_rows):
            return [_row_unit(src, dst, sem, r, unit_rows) for r in range(0, nrows, unit_rows)]

        wqb_ur = max(8, UB // (HD * 2))
        u_wqb = [_col_unit(wqb_hbm, wqb_v, sem_w.at[2], r, wqb_ur, HD) for r in range(0, M, wqb_ur)]
        u_wqb = _merge(u_wqb[:len(u_wqb) // 2], u_wqb[len(u_wqb) // 2:])
        u_wqa = rows_units(wqa_hbm, wqa_v, sem_w.at[3], M * H, UR)
        u_wuk = rows_units(wuk_hbm, wuk_v, sem_w.at[3], Dc * H, UR)
        u_ckv = rows_units(ckv_hbm.at[0], ckv_v, sem_w.at[4], Sk, UB // (Dc * 2))
        u_wuv = rows_units(wuv_hbm, wuv_v, sem_w.at[4], Dc * H, UR)
        u_t1 = _merge(u_wqa, u_wuk)
        u_t2 = _merge(u_ckv, u_wuv)
        u_t3 = []
        r = 0
        for gi, n in enumerate(WO_GROUPS):
            for _ in range(n):
                u_t3.append(_row_unit(woa_hbm, woa_v, sem_o.at[gi], r, WO_UR))
                u_t3.append(_row_unit(wob_hbm, wob_v, sem_o.at[gi], r, WO_UR))
                r += WO_UR

        def head_units(h, slot):
            out = []
            for j in range(UPH):
                out.append(_row_unit(k_hbm.at[0, h], kbuf.at[slot], sem_k.at[slot], j * UR, UR))
                out.append(_row_unit(v_hbm.at[0, h], vbuf.at[slot], sem_v.at[slot], j * UR, UR))
            return out

        def advance(seq, i):
            if i % HB == 0:
                for k in range(i, min(i + HB, len(seq))):
                    if k < seq_lim[0]:
                        seq[k].wait_hi()
            seq[i].wait_lo()
            if i + W0 < len(seq):
                seq[i + W0].start_hi()
            if i + W < len(seq):
                seq[i + W].start_lo()

        seq_lim = [0]

        def advance_n(seq, i0, n):
            for k in range(n):
                advance(seq, i0 + k)

        pro = u_wqb
        for h in range(32 - HN, 32 - HN + LOOK):
            pro = pro + head_units(h, h % NBUF)
        npro = len(u_wqb)
        assert npro >= W and HB <= W0

        cp_x.start(priority=PQ0)
        cp_gw.start(priority=PQ0)
        for i in range(W0):
            pro[i].start_hi()
        for i in range(W):
            pro[i].start_lo()

        e_row = lax.broadcasted_iota(jnp.int32, (128, HD), 0)
        e_col = lax.broadcasted_iota(jnp.int32, (128, HD), 1)
        e0 = jnp.where(e_row == (e_col >> 5), 1.0, 0.0).astype(_BF16)
        d_row = lax.broadcasted_iota(jnp.int32, (H, HD), 0)
        d_col = lax.broadcasted_iota(jnp.int32, (H, HD), 1)
        diag = (d_col & (H - 1)) == d_row

        cp_x.wait()
        cp_gw.wait()
        x = x_v[0].astype(_F32)
        gw = gw_v[...].astype(_F32).reshape(1, M)
        g = jax.nn.sigmoid(jnp.sum(x * gw, axis=-1, keepdims=True))
        x8 = jnp.broadcast_to(x, (8, M)).astype(_BF16)

        assert npro % HB == 0 and UH % HB == 0
        seq_lim[0] = npro
        advance_n(pro, 0, npro)
        qb = _dot(x8, wqb_v[...]) * scale
        for h in range(H):
            qb_s[h] = qb[:, h * D:(h + 1) * D]

        def attend(h, slot):
            if SKIP_COMPUTE:
                ob_s[h] = qb_s[h]
                return
            q = qb_s[h].astype(_BF16)
            s = _dot_nt(q, kbuf[slot])
            m = jnp.max(s, axis=-1, keepdims=True)
            p = jnp.exp(s - m)
            l = jnp.sum(p, axis=-1, keepdims=True)
            o = _dot(p.astype(_BF16), vbuf[slot])
            ob_s[h] = o / l

        def body(h, carry):
            seq = []
            for k in range(LOOK + 1):
                seq = seq + head_units(h + k, lax.rem(h + k, NBUF))
            seq_lim[0] = UH
            advance_n(seq, 0, UH)
            attend(h, lax.rem(h, NBUF))
            return carry

        lax.fori_loop(32 - HN, H - LOOK, body, 0)

        end = []
        for h in range(H - LOOK, H):
            end = end + head_units(h, h % NBUF)
        end = end + u_t1 + u_t2 + u_t3
        pos = [0]

        seq_lim[0] = len(end)

        def adv_end(n):
            n = min(n, len(end) - pos[0])
            advance_n(end, pos[0], n)
            pos[0] += n

        def adv_to(target):
            adv_end(max(0, target - pos[0]))

        def tick(n):
            adv_end(n * TICK // 4)

        p_t1 = LOOK * UH + len(u_t1)
        p_t2 = p_t1 + len(u_t2)

        for h in range(H - LOOK, H):
            adv_end(UH)
            attend(h, h % NBUF)

        if SKIP_A:
            adv_end(len(end) - pos[0])
            o_ref[0] = (x * g + ob_s[3][0:1, 0:1]).astype(o_ref.dtype)
            return
        x5 = jnp.concatenate(
            [x[:, c * 128:(c + 1) * 128] for c in range(NXC)]
            + [jnp.zeros((8 - NXC, 128), _F32)], axis=0).astype(_BF16)
        xr = _dot(x5, e0)
        adv_to(p_t1)
        qa = jnp.zeros((H, D), _F32)
        for c in range(NXC):
            sc = jnp.where(diag, jnp.broadcast_to(xr[c:c + 1, :], (H, HD)), 0.0).astype(_BF16)
            qa = qa + _dot(sc, wqa_v[pl.ds(c * HD, HD), :])
            tick(1)
        qa = (qa * scale).astype(_BF16)

        qabs = []
        for b in range(NCB):
            t = _dot_nt(qa, wuk_v[pl.ds(b * HD, HD), :])
            mb = jnp.where(diag, t, 0.0).astype(_BF16)
            tick(2)
            qabs.append(_dot_nt(mb, e0))
            tick(2)
        qabs = jnp.concatenate(qabs, axis=1).astype(_BF16)

        adv_to(p_t2)
        KB = Sk // 4
        s = []
        for kb in range(4):
            s.append(_dot_nt(qabs, ckv_v[pl.ds(kb * KB, KB), :]))
            tick(1)
        s = jnp.concatenate(s, axis=1)
        m = jnp.max(s, axis=-1, keepdims=True)
        p = jnp.exp(s - m)
        l = jnp.sum(p, axis=-1, keepdims=True)
        p = p.astype(_BF16)
        tick(1)
        cl = jnp.zeros((H, Dc), _F32)
        for kb in range(4):
            cl = cl + _dot(p[:, kb * KB:(kb + 1) * KB], ckv_v[pl.ds(kb * KB, KB), :])
            tick(1)
        cl = (cl / l).astype(_BF16)

        ctx = jnp.zeros((H, D), _F32)
        for b in range(NCB):
            xb = _dot(cl[:, b * 128:(b + 1) * 128], e0)
            sb = jnp.where(diag, xb, 0.0).astype(_BF16)
            ctx = ctx + _dot(sb, wuv_v[pl.ds(b * HD, HD), :])
            tick(2)

        sub = lax.broadcasted_iota(jnp.int32, (8, D), 0)
        ctx_flat = jnp.concatenate(
            [jnp.where(sub == (h % 8), ctx[8 * (h // 8):8 * (h // 8) + 8, :], 0.0) for h in range(H)],
            axis=1).astype(_BF16)
        o_flat = jnp.concatenate([ob_s[h] for h in range(H)], axis=1).astype(_BF16)
        one_g = 1.0 - g

        acc_a = jnp.zeros((8, M), _F32)
        acc_b = jnp.zeros((8, M), _F32)
        o = 0
        target = p_t2
        for n in WO_GROUPS:
            target += 2 * n
            adv_to(target)
            n = n * WO_UR
            acc_a = acc_a + _dot(ctx_flat[:, o:o + n], woa_v[pl.ds(o, n), :])
            acc_b = acc_b + _dot(o_flat[:, o:o + n], wob_v[pl.ds(o, n), :])
            o += n
        assert pos[0] == len(end)
        a = jnp.sum(acc_a, axis=0, keepdims=True)
        o_ref[0] = (g * a + one_g * acc_b[0:1, :]).astype(o_ref.dtype)

    any_spec = pl.BlockSpec(memory_space=pl.ANY)
    scratch = [
        pltpu.VMEM((1, 1, M), _BF16),
        pltpu.VMEM((M,), _BF16),
        pltpu.VMEM((M, HD), _BF16),
        pltpu.VMEM((NBUF, Sk, D), _BF16),
        pltpu.VMEM((NBUF, Sk, D), _BF16),
        pltpu.VMEM((M * H, D), _BF16),
        pltpu.VMEM((Dc * H, D), _BF16),
        pltpu.VMEM((Sk, Dc), _BF16),
        pltpu.VMEM((Dc * H, D), _BF16),
        pltpu.VMEM((HD, M), _BF16),
        pltpu.VMEM((HD, M), _BF16),
        pltpu.VMEM((H, 8, D), _F32),
        pltpu.VMEM((H, 8, D), _F32),
        pltpu.SemaphoreType.DMA((5,)),
        pltpu.SemaphoreType.DMA((NBUF,)),
        pltpu.SemaphoreType.DMA((NBUF,)),
        pltpu.SemaphoreType.DMA((len(WO_GROUPS),)),
    ]
    return pl.pallas_call(
        kernel,
        out_shape=jax.ShapeDtypeStruct((B, Sq, M), A_x.dtype),
        in_specs=[any_spec] * 11,
        out_specs=pl.BlockSpec(memory_space=pltpu.VMEM),
        scratch_shapes=scratch,
        compiler_params=pltpu.CompilerParams(
            vmem_limit_bytes=100 * 1024 * 1024,
            disable_semaphore_checks=NOSEM, disable_bounds_checks=NOBND),
    )(A_x, gate_w, B_wq, B_k_cache, B_v_cache, w_q2, w_uk2, A_c_kv, w_uv2, w_o2, B_wo)
```

```python
import jax
import jax.numpy as jnp
from jax import lax
import jax.experimental.pallas as pl
import jax.experimental.pallas.tpu as pltpu

_NT = (((1,), (1,)), ((), ()))
_F32 = jnp.float32
_BF16 = jnp.bfloat16

UPH = 16
Q0_NUM, Q0_DEN = 3, 8
WLO = 40
WHI = 16
TICK = 8
HB = 8
WO_GROUPS = (8, 8, 8, 4, 2, 1, 1)
NOSEM = True
NOBND = True
PQ0, PQ1 = 0, 1
SKIP_COMPUTE = False
SKIP_A = False
HN = 32


def _dot(a, b):
    return jnp.dot(a, b, preferred_element_type=_F32)


def _dot_nt(a, b):
    return lax.dot_general(a, b, _NT, preferred_element_type=_F32)


class _Unit:
    def __init__(self, hi, lo):
        self.hi, self.lo = hi, lo

    def start_hi(self):
        if self.hi is not None:
            self.hi().start(priority=PQ0)

    def start_lo(self):
        self.lo().start(priority=PQ1)

    def wait_hi(self):
        if self.hi is not None:
            self.hi().wait()

    def wait_lo(self):
        self.lo().wait()


def _row_unit(src, dst, sem, r0, n):
    nh = (n * Q0_NUM // Q0_DEN) // 16 * 16
    until = lambda a, k: pltpu.make_async_copy(src.at[pl.ds(a, k)], dst.at[pl.ds(a, k)], sem)
    if nh == 0:
        return _Unit(None, lambda: until(r0, n))
    return _Unit(lambda: until(r0, nh), lambda: until(r0 + nh, n - nh))


def _col_unit(src, dst, sem, r0, n, ncols):
    ch = (ncols * Q0_NUM // Q0_DEN) // 128 * 128
    until = lambda a, k: pltpu.make_async_copy(
        src.at[pl.ds(r0, n), pl.ds(a, k)], dst.at[pl.ds(r0, n), pl.ds(a, k)], sem)
    if ch == 0:
        return _Unit(None, lambda: until(0, ncols))
    return _Unit(lambda: until(0, ch), lambda: until(ch, ncols - ch))


def _merge(a, b):
    out, i, j = [], 0, 0
    while i < len(a) or j < len(b):
        if j >= len(b) or (i < len(a) and i * len(b) <= j * len(a)):
            out.append(a[i]); i += 1
        else:
            out.append(b[j]); j += 1
    return out


@jax.jit
def pallas_gated_mix__compressed_kv_cla__gqa_block_cached__decode_kernel(
    A_x: jax.Array,
    A_c_kv: jax.Array,
    A_w_q: jax.Array,
    A_w_uk: jax.Array,
    A_w_uv: jax.Array,
    A_w_o: jax.Array,
    B_x: jax.Array,
    B_k_cache: jax.Array,
    B_v_cache: jax.Array,
    B_wq: jax.Array,
    B_wo: jax.Array,
    gate_w: jax.Array,
):
    B, Sq, M = A_x.shape
    _, Sk, Dc = A_c_kv.shape
    _, H, D = A_w_q.shape
    assert B == 1 and Sq == 1 and D == 128 and H == 32
    assert B_k_cache.shape == (1, H, Sk, D) and B_v_cache.shape == (1, H, Sk, D)
    HD = H * D
    scale = float(D) ** -0.5
    NXC = M // 128
    NCB = Dc // 128
    LOOK = -(-WLO // (2 * UPH))
    NBUF = LOOK + 1
    UR = Sk // UPH
    UB = UR * D * 2
    UH = 2 * UPH
    W, W0 = WLO, WHI
    assert W0 <= W
    WO_UR = HD // sum(WO_GROUPS)

    w_q2 = A_w_q.reshape(M * H, D)
    w_uk2 = A_w_uk.reshape(Dc * H, D)
    w_uv2 = A_w_uv.reshape(Dc * H, D)
    w_o2 = A_w_o.reshape(HD, M)

    def kernel(x_hbm, gw_hbm, wqb_hbm, k_hbm, v_hbm, wqa_hbm, wuk_hbm, ckv_hbm,
               wuv_hbm, woa_hbm, wob_hbm,
               o_ref,
               x_v, gw_v, wqb_v, kbuf, vbuf, wqa_v, wuk_v, ckv_v, wuv_v, woa_v, wob_v,
               qb_s, ob_s,
               sem_w, sem_k, sem_v, sem_o):
        cp_x = pltpu.make_async_copy(x_hbm, x_v, sem_w.at[0])
        cp_gw = pltpu.make_async_copy(gw_hbm, gw_v, sem_w.at[1])

        def rows_units(src, dst, sem, nrows, unit_rows):
            return [_row_unit(src, dst, sem, r, unit_rows) for r in range(0, nrows, unit_rows)]

        wqb_ur = max(8, UB // (HD * 2))
        u_wqb = [_col_unit(wqb_hbm, wqb_v, sem_w.at[2], r, wqb_ur, HD) for r in range(0, M, wqb_ur)]
        u_wqb = _merge(u_wqb[:len(u_wqb) // 2], u_wqb[len(u_wqb) // 2:])
        u_wqa = rows_units(wqa_hbm, wqa_v, sem_w.at[3], M * H, UR)
        u_wuk = rows_units(wuk_hbm, wuk_v, sem_w.at[3], Dc * H, UR)
        u_ckv = rows_units(ckv_hbm.at[0], ckv_v, sem_w.at[4], Sk, UB // (Dc * 2))
        u_wuv = rows_units(wuv_hbm, wuv_v, sem_w.at[4], Dc * H, UR)
        u_t1 = _merge(u_wqa, u_wuk)
        u_t2 = _merge(u_ckv, u_wuv)
        u_t3 = []
        r = 0
        for gi, n in enumerate(WO_GROUPS):
            for _ in range(n):
                u_t3.append(_row_unit(woa_hbm, woa_v, sem_o.at[gi], r, WO_UR))
                u_t3.append(_row_unit(wob_hbm, wob_v, sem_o.at[gi], r, WO_UR))
                r += WO_UR

        def head_units(h, slot):
            out = []
            for j in range(UPH):
                out.append(_row_unit(k_hbm.at[0, h], kbuf.at[slot], sem_k.at[slot], j * UR, UR))
                out.append(_row_unit(v_hbm.at[0, h], vbuf.at[slot], sem_v.at[slot], j * UR, UR))
            return out

        def advance(seq, i):
            if i % HB == 0:
                for k in range(i, min(i + HB, len(seq))):
                    if k < seq_lim[0]:
                        seq[k].wait_hi()
            seq[i].wait_lo()
            if i + W0 < len(seq):
                seq[i + W0].start_hi()
            if i + W < len(seq):
                seq[i + W].start_lo()

        seq_lim = [0]

        def advance_n(seq, i0, n):
            for k in range(n):
                advance(seq, i0 + k)

        pro = u_wqb
        for h in range(32 - HN, 32 - HN + LOOK):
            pro = pro + head_units(h, h % NBUF)
        npro = len(u_wqb)
        assert npro >= W and HB <= W0

        cp_x.start(priority=PQ0)
        cp_gw.start(priority=PQ0)
        for i in range(W0):
            pro[i].start_hi()
        for i in range(W):
            pro[i].start_lo()

        e_row = lax.broadcasted_iota(jnp.int32, (128, HD), 0)
        e_col = lax.broadcasted_iota(jnp.int32, (128, HD), 1)
        e0 = jnp.where(e_row == (e_col >> 5), 1.0, 0.0).astype(_BF16)
        d_row = lax.broadcasted_iota(jnp.int32, (H, HD), 0)
        d_col = lax.broadcasted_iota(jnp.int32, (H, HD), 1)
        diag = (d_col & (H - 1)) == d_row

        cp_x.wait()
        cp_gw.wait()
        x = x_v[0].astype(_F32)
        gw = gw_v[...].astype(_F32).reshape(1, M)
        g = jax.nn.sigmoid(jnp.sum(x * gw, axis=-1, keepdims=True))
        x8 = jnp.broadcast_to(x, (8, M)).astype(_BF16)

        assert npro % HB == 0 and UH % HB == 0
        seq_lim[0] = npro
        advance_n(pro, 0, npro)
        qb = _dot(x8, wqb_v[...]) * scale
        for h in range(H):
            qb_s[h] = qb[:, h * D:(h + 1) * D]

        def attend(h, slot):
            if SKIP_COMPUTE:
                ob_s[h] = qb_s[h]
                return
            q = qb_s[h].astype(_BF16)
            s = _dot_nt(q, kbuf[slot])
            m = jnp.max(s, axis=-1, keepdims=True)
            p = jnp.exp(s - m)
            l = jnp.sum(p, axis=-1, keepdims=True)
            o = _dot(p.astype(_BF16), vbuf[slot])
            ob_s[h] = o / l

        def body(h, carry):
            seq = []
            for k in range(LOOK + 1):
                seq = seq + head_units(h + k, lax.rem(h + k, NBUF))
            seq_lim[0] = UH
            advance_n(seq, 0, UH)
            attend(h, lax.rem(h, NBUF))
            return carry

        lax.fori_loop(32 - HN, H - LOOK, body, 0)

        end = []
        for h in range(H - LOOK, H):
            end = end + head_units(h, h % NBUF)
        end = end + u_t1 + u_t2 + u_t3
        pos = [0]

        seq_lim[0] = len(end)

        def adv_end(n):
            n = min(n, len(end) - pos[0])
            advance_n(end, pos[0], n)
            pos[0] += n

        def adv_to(target):
            adv_end(max(0, target - pos[0]))

        def tick(n):
            adv_end(n * TICK // 4)

        p_t1 = LOOK * UH + len(u_t1)
        p_t2 = p_t1 + len(u_t2)

        for h in range(H - LOOK, H):
            adv_end(UH)
            attend(h, h % NBUF)

        if SKIP_A:
            adv_end(len(end) - pos[0])
            o_ref[0] = (x * g + ob_s[3][0:1, 0:1]).astype(o_ref.dtype)
            return
        x5 = jnp.concatenate(
            [x[:, c * 128:(c + 1) * 128] for c in range(NXC)]
            + [jnp.zeros((8 - NXC, 128), _F32)], axis=0).astype(_BF16)
        xr = _dot(x5, e0)
        adv_to(p_t1)
        qa = jnp.zeros((H, D), _F32)
        for c in range(NXC):
            sc = jnp.where(diag, jnp.broadcast_to(xr[c:c + 1, :], (H, HD)), 0.0).astype(_BF16)
            qa = qa + _dot(sc, wqa_v[pl.ds(c * HD, HD), :])
            tick(1)
        qa = (qa * scale).astype(_BF16)

        qabs = []
        for b in range(NCB):
            t = _dot_nt(qa, wuk_v[pl.ds(b * HD, HD), :])
            mb = jnp.where(diag, t, 0.0).astype(_BF16)
            tick(2)
            qabs.append(_dot_nt(mb, e0))
            tick(2)
        qabs = jnp.concatenate(qabs, axis=1).astype(_BF16)

        adv_to(p_t2)
        KB = Sk // 4
        s = []
        for kb in range(4):
            s.append(_dot_nt(qabs, ckv_v[pl.ds(kb * KB, KB), :]))
            tick(1)
        s = jnp.concatenate(s, axis=1)
        m = jnp.max(s, axis=-1, keepdims=True)
        p = jnp.exp(s - m)
        l = jnp.sum(p, axis=-1, keepdims=True)
        p = p.astype(_BF16)
        tick(1)
        cl = jnp.zeros((H, Dc), _F32)
        for kb in range(4):
            cl = cl + _dot(p[:, kb * KB:(kb + 1) * KB], ckv_v[pl.ds(kb * KB, KB), :])
            tick(1)
        cl = (cl / l).astype(_BF16)

        ctx = jnp.zeros((H, D), _F32)
        for b in range(NCB):
            xb = _dot(cl[:, b * 128:(b + 1) * 128], e0)
            sb = jnp.where(diag, xb, 0.0).astype(_BF16)
            ctx = ctx + _dot(sb, wuv_v[pl.ds(b * HD, HD), :])
            tick(2)

        sub = lax.broadcasted_iota(jnp.int32, (8, D), 0)
        ctx_flat = jnp.concatenate(
            [jnp.where(sub == (h % 8), ctx[8 * (h // 8):8 * (h // 8) + 8, :], 0.0) for h in range(H)],
            axis=1).astype(_BF16)
        o_flat = jnp.concatenate([ob_s[h] for h in range(H)], axis=1).astype(_BF16)
        one_g = 1.0 - g

        acc_a = jnp.zeros((8, M), _F32)
        acc_b = jnp.zeros((8, M), _F32)
        o = 0
        target = p_t2
        for n in WO_GROUPS:
            target += 2 * n
            adv_to(target)
            n = n * WO_UR
            acc_a = acc_a + _dot(ctx_flat[:, o:o + n], woa_v[pl.ds(o, n), :])
            acc_b = acc_b + _dot(o_flat[:, o:o + n], wob_v[pl.ds(o, n), :])
            o += n
        assert pos[0] == len(end)
        a = jnp.sum(acc_a, axis=0, keepdims=True)
        o_ref[0] = (g * a + one_g * acc_b[0:1, :]).astype(o_ref.dtype)

    any_spec = pl.BlockSpec(memory_space=pl.ANY)
    scratch = [
        pltpu.VMEM((1, 1, M), _BF16),
        pltpu.VMEM((M,), _BF16),
        pltpu.VMEM((M, HD), _BF16),
        pltpu.VMEM((NBUF, Sk, D), _BF16),
        pltpu.VMEM((NBUF, Sk, D), _BF16),
        pltpu.VMEM((M * H, D), _BF16),
        pltpu.VMEM((Dc * H, D), _BF16),
        pltpu.VMEM((Sk, Dc), _BF16),
        pltpu.VMEM((Dc * H, D), _BF16),
        pltpu.VMEM((HD, M), _BF16),
        pltpu.VMEM((HD, M), _BF16),
        pltpu.VMEM((H, 8, D), _F32),
        pltpu.VMEM((H, 8, D), _F32),
        pltpu.SemaphoreType.DMA((5,)),
        pltpu.SemaphoreType.DMA((NBUF,)),
        pltpu.SemaphoreType.DMA((NBUF,)),
        pltpu.SemaphoreType.DMA((len(WO_GROUPS),)),
    ]
    return pl.pallas_call(
        kernel,
        out_shape=jax.ShapeDtypeStruct((B, Sq, M), A_x.dtype),
        in_specs=[any_spec] * 11,
        out_specs=pl.BlockSpec(memory_space=pltpu.VMEM),
        scratch_shapes=scratch,
        compiler_params=pltpu.CompilerParams(
            vmem_limit_bytes=100 * 1024 * 1024,
            disable_semaphore_checks=NOSEM, disable_bounds_checks=NOBND),
    )(A_x, gate_w, B_wq, B_k_cache, B_v_cache, w_q2, w_uk2, A_c_kv, w_uv2, w_o2, B_wo)
```

```python
import jax
import jax.numpy as jnp
from jax import lax
import jax.experimental.pallas as pl
import jax.experimental.pallas.tpu as pltpu

_NT = (((1,), (1,)), ((), ()))
_F32 = jnp.float32
_BF16 = jnp.bfloat16

PERIOD = 64 * 1024
PHI = dict(kv=30, wqb=30, wqa=28, wuk=28, ckv=32, wuv=28, woa=30, wob=30)
WLO = 56
WHI = 32
TICK = 16
W0_WQ = W0_T1 = W0_T2 = W0_T3 = None
HB = 8
WO_GROUPS = (1024, 1024, 1024, 512, 256, 128, 128)
NOSEM = True
NOBND = True
PQ0, PQ1 = 0, 1
SKIP_COMPUTE = False
SKIP_A = False
HN = 32


def _dot(a, b):
    return jnp.dot(a, b, preferred_element_type=_F32)


def _dot_nt(a, b):
    return lax.dot_general(a, b, _NT, preferred_element_type=_F32)


class _Unit:
    def __init__(self, hi, lo):
        self.hi, self.lo = hi, lo
        self.w0 = WHI

    def start_hi(self):
        if self.hi is not None:
            self.hi().start(priority=PQ0)

    def start_lo(self):
        self.lo().start(priority=PQ1)

    def wait_hi(self):
        if self.hi is not None:
            self.hi().wait()

    def wait_lo(self):
        self.lo().wait()


def _row_units(src, dst, sem_of_row, nrows, row_bytes, phi_kib):
    tb = 8 * row_bytes
    near = lambda off: min(nrows, 8 * ((off + tb // 2) // tb))
    out = []
    k = 0
    while near(k * PERIOD) < nrows:
        a, m, b = near(k * PERIOD), near(k * PERIOD + phi_kib * 1024), near((k + 1) * PERIOD)
        sem = sem_of_row(a)
        mk = lambda r, n, q, sem=sem: (lambda: pltpu.make_async_copy(
            src.at[pl.ds(r, n)], dst.at[pl.ds(r, n)], sem[q]))
        if m >= b:
            u = _Unit(None, mk(a, b - a, 1))
        elif m <= a:
            u = _Unit(None, mk(a, b - a, 1))
        else:
            u = _Unit(mk(a, m - a, 0), mk(m, b - m, 1))
        u.row0 = a
        out.append(u)
        k += 1
    return out


def _col_unit(src, dst, sem, r0, n, ncols, ch):
    until = lambda a, k, q: pltpu.make_async_copy(
        src.at[pl.ds(r0, n), pl.ds(a, k)], dst.at[pl.ds(r0, n), pl.ds(a, k)], sem[q])
    return _Unit(lambda: until(0, ch, 0), lambda: until(ch, ncols - ch, 1))


def _merge(a, b):
    out, i, j = [], 0, 0
    while i < len(a) or j < len(b):
        if j >= len(b) or (i < len(a) and i * len(b) <= j * len(a)):
            out.append(a[i]); i += 1
        else:
            out.append(b[j]); j += 1
    return out


@jax.jit
def pallas_gated_mix__compressed_kv_cla__gqa_block_cached__decode_kernel(
    A_x: jax.Array,
    A_c_kv: jax.Array,
    A_w_q: jax.Array,
    A_w_uk: jax.Array,
    A_w_uv: jax.Array,
    A_w_o: jax.Array,
    B_x: jax.Array,
    B_k_cache: jax.Array,
    B_v_cache: jax.Array,
    B_wq: jax.Array,
    B_wo: jax.Array,
    gate_w: jax.Array,
):
    B, Sq, M = A_x.shape
    _, Sk, Dc = A_c_kv.shape
    _, H, D = A_w_q.shape
    assert B == 1 and Sq == 1 and D == 128 and H == 32
    assert B_k_cache.shape == (1, H, Sk, D) and B_v_cache.shape == (1, H, Sk, D)
    HD = H * D
    scale = float(D) ** -0.5
    NXC = M // 128
    NCB = Dc // 128
    UPH = Sk * D * 2 // PERIOD
    LOOK = -(-WLO // (2 * UPH))
    NBUF = LOOK + 1
    UH = 2 * UPH
    W, W0 = WLO, WHI
    assert W0 <= W
    assert sum(WO_GROUPS) == HD

    w_q2 = A_w_q.reshape(M * H, D)
    w_uk2 = A_w_uk.reshape(Dc * H, D)
    w_uv2 = A_w_uv.reshape(Dc * H, D)
    w_o2 = A_w_o.reshape(HD, M)

    def kernel(x_hbm, gw_hbm, wqb_hbm, k_hbm, v_hbm, wqa_hbm, wuk_hbm, ckv_hbm,
               wuv_hbm, woa_hbm, wob_hbm,
               o_ref,
               x_v, gw_v, wqb_v, kbuf, vbuf, wqa_v, wuk_v, ckv_v, wuv_v, woa_v, wob_v,
               qb_s, ob_s,
               sem_w, sem_k, sem_v, sem_o):
        def pair(sem, idx):
            return (sem.at[0 if True else 1, idx], sem.at[1, idx])

        cp_x = pltpu.make_async_copy(x_hbm, x_v, sem_w.at[0, 0])
        cp_gw = pltpu.make_async_copy(gw_hbm, gw_v, sem_w.at[0, 1])

        assert HD * 2 * 8 == PERIOD
        u_wqb = [_col_unit(wqb_hbm, wqb_v, pair(sem_w, 2), r, 8, HD, PHI['wqb'] * 64)
                 for r in range(0, M, 8)]
        u_wqb = _merge(u_wqb[:len(u_wqb) // 2], u_wqb[len(u_wqb) // 2:])
        u_wqa = _row_units(wqa_hbm, wqa_v, lambda r: pair(sem_w, 3), M * H, 2 * D, PHI['wqa'])
        u_wuk = _row_units(wuk_hbm, wuk_v, lambda r: pair(sem_w, 3), Dc * H, 2 * D, PHI['wuk'])
        u_ckv = _row_units(ckv_hbm.at[0], ckv_v, lambda r: pair(sem_w, 4), Sk, 2 * Dc, PHI['ckv'])
        u_wuv = _row_units(wuv_hbm, wuv_v, lambda r: pair(sem_w, 4), Dc * H, 2 * D, PHI['wuv'])
        u_t1 = _merge(u_wqa, u_wuk)
        u_t2 = _merge(u_ckv, u_wuv)
        wo_start = [sum(WO_GROUPS[:i]) for i in range(len(WO_GROUPS))]
        grp = lambda r: max(i for i, o in enumerate(wo_start) if o <= r)
        u_woa = _row_units(woa_hbm, woa_v, lambda r: pair(sem_o, grp(r)), HD, 2 * M, PHI['woa'])
        u_wob = _row_units(wob_hbm, wob_v, lambda r: pair(sem_o, grp(r)), HD, 2 * M, PHI['wob'])
        t3_groups = [_merge([u for u in u_woa if grp(u.row0) == gi], [u for u in u_wob if grp(u.row0) == gi])
                     for gi in range(len(WO_GROUPS))]
        u_t3 = [u for gr in t3_groups for u in gr]
        for us, w0 in ((u_wqb, W0_WQ), (u_t1, W0_T1), (u_t2, W0_T2), (u_t3, W0_T3)):
            for u in us:
                u.w0 = w0 or WHI

        def head_units(h, slot):
            uk = _row_units(k_hbm.at[0, h], kbuf.at[slot], lambda r: pair(sem_k, slot), Sk, 2 * D, PHI['kv'])
            uv = _row_units(v_hbm.at[0, h], vbuf.at[slot], lambda r: pair(sem_v, slot), Sk, 2 * D, PHI['kv'])
            return [u for kv in zip(uk, uv) for u in kv]

        def advance(seq, i):
            if i % HB == 0:
                for k in range(i, min(i + HB, len(seq))):
                    if k < seq_lim[0]:
                        seq[k].wait_hi()
            seq[i].wait_lo()
            for k in range(i + 1, min(i + W + 1, len(seq))):
                if seq[k].w0 == k - i:
                    seq[k].start_hi()
            if i + W < len(seq):
                seq[i + W].start_lo()

        seq_lim = [0]

        def advance_n(seq, i0, n):
            for k in range(n):
                advance(seq, i0 + k)

        pro = u_wqb
        for h in range(32 - HN, 32 - HN + LOOK):
            pro = pro + head_units(h, h % NBUF)
        npro = len(u_wqb)
        assert npro >= W

        cp_x.start(priority=PQ0)
        cp_gw.start(priority=PQ0)
        for i in range(W):
            if i < pro[i].w0:
                pro[i].start_hi()
        for i in range(W):
            pro[i].start_lo()

        e_row = lax.broadcasted_iota(jnp.int32, (128, HD), 0)
        e_col = lax.broadcasted_iota(jnp.int32, (128, HD), 1)
        e0 = jnp.where(e_row == (e_col >> 5), 1.0, 0.0).astype(_BF16)
        d_row = lax.broadcasted_iota(jnp.int32, (H, HD), 0)
        d_col = lax.broadcasted_iota(jnp.int32, (H, HD), 1)
        diag = (d_col & (H - 1)) == d_row

        cp_x.wait()
        cp_gw.wait()
        x = x_v[0].astype(_F32)
        gw = gw_v[...].astype(_F32).reshape(1, M)
        g = jax.nn.sigmoid(jnp.sum(x * gw, axis=-1, keepdims=True))
        x8 = jnp.broadcast_to(x, (8, M)).astype(_BF16)

        assert npro % HB == 0 and UH % HB == 0
        seq_lim[0] = npro
        advance_n(pro, 0, npro)
        qb = _dot(x8, wqb_v[...]) * scale
        for h in range(H):
            qb_s[h] = qb[:, h * D:(h + 1) * D]

        def attend(h, slot):
            if SKIP_COMPUTE:
                ob_s[h] = qb_s[h]
                return
            q = qb_s[h].astype(_BF16)
            s = _dot_nt(q, kbuf[slot])
            m = jnp.max(s, axis=-1, keepdims=True)
            p = jnp.exp(s - m)
            l = jnp.sum(p, axis=-1, keepdims=True)
            o = _dot(p.astype(_BF16), vbuf[slot])
            ob_s[h] = o / l

        def body(h, carry):
            seq = []
            for k in range(LOOK + 1):
                seq = seq + head_units(h + k, lax.rem(h + k, NBUF))
            seq_lim[0] = UH
            advance_n(seq, 0, UH)
            attend(h, lax.rem(h, NBUF))
            return carry

        lax.fori_loop(32 - HN, H - LOOK, body, 0)

        end = []
        for h in range(H - LOOK, H):
            end = end + head_units(h, h % NBUF)
        end = end + u_t1 + u_t2 + u_t3
        pos = [0]

        seq_lim[0] = len(end)

        def adv_end(n):
            n = min(n, len(end) - pos[0])
            advance_n(end, pos[0], n)
            pos[0] += n

        def adv_to(target):
            adv_end(max(0, target - pos[0]))

        def tick(n):
            adv_end(n * TICK // 4)

        p_t1 = LOOK * UH + len(u_t1)
        p_t2 = p_t1 + len(u_t2)

        for h in range(H - LOOK, H):
            adv_end(UH)
            attend(h, h % NBUF)

        if SKIP_A:
            adv_end(len(end) - pos[0])
            o_ref[0] = (x * g + ob_s[3][0:1, 0:1]).astype(o_ref.dtype)
            return
        x5 = jnp.concatenate(
            [x[:, c * 128:(c + 1) * 128] for c in range(NXC)]
            + [jnp.zeros((8 - NXC, 128), _F32)], axis=0).astype(_BF16)
        xr = _dot(x5, e0)
        adv_to(p_t1)
        qa = jnp.zeros((H, D), _F32)
        for c in range(NXC):
            sc = jnp.where(diag, jnp.broadcast_to(xr[c:c + 1, :], (H, HD)), 0.0).astype(_BF16)
            qa = qa + _dot(sc, wqa_v[pl.ds(c * HD, HD), :])
            tick(1)
        qa = (qa * scale).astype(_BF16)

        qabs = []
        for b in range(NCB):
            t = _dot_nt(qa, wuk_v[pl.ds(b * HD, HD), :])
            mb = jnp.where(diag, t, 0.0).astype(_BF16)
            tick(2)
            qabs.append(_dot_nt(mb, e0))
            tick(2)
        qabs = jnp.concatenate(qabs, axis=1).astype(_BF16)

        adv_to(p_t2)
        KB = Sk // 4
        s = []
        for kb in range(4):
            s.append(_dot_nt(qabs, ckv_v[pl.ds(kb * KB, KB), :]))
            tick(1)
        s = jnp.concatenate(s, axis=1)
        m = jnp.max(s, axis=-1, keepdims=True)
        p = jnp.exp(s - m)
        l = jnp.sum(p, axis=-1, keepdims=True)
        p = p.astype(_BF16)
        tick(1)
        cl = jnp.zeros((H, Dc), _F32)
        for kb in range(4):
            cl = cl + _dot(p[:, kb * KB:(kb + 1) * KB], ckv_v[pl.ds(kb * KB, KB), :])
            tick(1)
        cl = (cl / l).astype(_BF16)

        ctx = jnp.zeros((H, D), _F32)
        for b in range(NCB):
            xb = _dot(cl[:, b * 128:(b + 1) * 128], e0)
            sb = jnp.where(diag, xb, 0.0).astype(_BF16)
            ctx = ctx + _dot(sb, wuv_v[pl.ds(b * HD, HD), :])
            tick(2)

        sub = lax.broadcasted_iota(jnp.int32, (8, D), 0)
        ctx_flat = jnp.concatenate(
            [jnp.where(sub == (h % 8), ctx[8 * (h // 8):8 * (h // 8) + 8, :], 0.0) for h in range(H)],
            axis=1).astype(_BF16)
        o_flat = jnp.concatenate([ob_s[h] for h in range(H)], axis=1).astype(_BF16)
        one_g = 1.0 - g

        acc_a = jnp.zeros((8, M), _F32)
        acc_b = jnp.zeros((8, M), _F32)
        o = 0
        target = p_t2
        for n, gr in zip(WO_GROUPS, t3_groups):
            target += len(gr)
            adv_to(target)
            acc_a = acc_a + _dot(ctx_flat[:, o:o + n], woa_v[pl.ds(o, n), :])
            acc_b = acc_b + _dot(o_flat[:, o:o + n], wob_v[pl.ds(o, n), :])
            o += n
        assert pos[0] == len(end)
        a = jnp.sum(acc_a, axis=0, keepdims=True)
        o_ref[0] = (g * a + one_g * acc_b[0:1, :]).astype(o_ref.dtype)

    any_spec = pl.BlockSpec(memory_space=pl.ANY)
    scratch = [
        pltpu.VMEM((1, 1, M), _BF16),
        pltpu.VMEM((M,), _BF16),
        pltpu.VMEM((M, HD), _BF16),
        pltpu.VMEM((NBUF, Sk, D), _BF16),
        pltpu.VMEM((NBUF, Sk, D), _BF16),
        pltpu.VMEM((M * H, D), _BF16),
        pltpu.VMEM((Dc * H, D), _BF16),
        pltpu.VMEM((Sk, Dc), _BF16),
        pltpu.VMEM((Dc * H, D), _BF16),
        pltpu.VMEM((HD, M), _BF16),
        pltpu.VMEM((HD, M), _BF16),
        pltpu.VMEM((H, 8, D), _F32),
        pltpu.VMEM((H, 8, D), _F32),
        pltpu.SemaphoreType.DMA((2, 5)),
        pltpu.SemaphoreType.DMA((2, NBUF)),
        pltpu.SemaphoreType.DMA((2, NBUF)),
        pltpu.SemaphoreType.DMA((2, len(WO_GROUPS))),
    ]
    return pl.pallas_call(
        kernel,
        out_shape=jax.ShapeDtypeStruct((B, Sq, M), A_x.dtype),
        in_specs=[any_spec] * 11,
        out_specs=pl.BlockSpec(memory_space=pltpu.VMEM),
        scratch_shapes=scratch,
        compiler_params=pltpu.CompilerParams(
            vmem_limit_bytes=100 * 1024 * 1024,
            disable_semaphore_checks=NOSEM, disable_bounds_checks=NOBND),
    )(A_x, gate_w, B_wq, B_k_cache, B_v_cache, w_q2, w_uk2, A_c_kv, w_uv2, w_o2, B_wo)
```

```python
import jax
import jax.numpy as jnp
from jax import lax
import jax.experimental.pallas as pl
import jax.experimental.pallas.tpu as pltpu

_NT = (((1,), (1,)), ((), ()))
_F32 = jnp.float32
_BF16 = jnp.bfloat16

PERIOD = 64 * 1024
PHI = dict(kv=30, wqb=30, wqa=28, wuk=28, ckv=32, wuv=28, woa=30, wob=30)
WLO = 56
DLT = 24
TICK = 6
HB = 8
WO_GROUPS = (1024, 1024, 1024, 512, 256, 128, 128)
NOSEM = True
NOBND = True
PQ0, PQ1 = 0, 1
SKIP_COMPUTE = False
SKIP_A = False
HN = 32
DROP = ()
WRAP = False
BARRIER = False
SPLITS = (6, 6, 6, 6, 6)


def _dot(a, b):
    return jnp.dot(a, b, preferred_element_type=_F32)


def _dot_nt(a, b):
    return lax.dot_general(a, b, _NT, preferred_element_type=_F32)


class _Unit:
    def __init__(self, hi, lo):
        self.hi, self.lo = hi, lo

    def start_hi(self):
        if self.hi is not None:
            self.hi().start(priority=PQ0)

    def start_lo(self):
        self.lo().start(priority=PQ1)

    def wait_hi(self):
        if self.hi is not None:
            self.hi().wait()

    def wait_lo(self):
        self.lo().wait()


def _row_units(src, dst, sem_of_row, nrows, row_bytes, phi_kib):
    tb = 8 * row_bytes
    near = lambda off: min(nrows, 8 * ((off + tb // 2) // tb))
    out = []
    k = 0
    while near(k * PERIOD) < nrows:
        a, m, b = near(k * PERIOD), near(k * PERIOD + phi_kib * 1024), near((k + 1) * PERIOD)
        sem = sem_of_row(a)
        mk = lambda r, n, q, sem=sem: (lambda: pltpu.make_async_copy(
            src.at[pl.ds(r, n)], dst.at[pl.ds(r, n)], sem[q]))
        if m >= b or m <= a:
            u = _Unit(None, mk(a, b - a, 1))
        else:
            u = _Unit(mk(a, m - a, 0), mk(m, b - m, 1))
        u.row0 = a
        out.append(u)
        k += 1
    return out


def _col_unit(src, dst, sem, r0, n, ncols, ch):
    until = lambda a, k, q: pltpu.make_async_copy(
        src.at[pl.ds(r0, n), pl.ds(a, k)], dst.at[pl.ds(r0, n), pl.ds(a, k)], sem[q])
    return _Unit(lambda: until(0, ch, 0), lambda: until(ch, ncols - ch, 1))


def _merge(a, b):
    out, i, j = [], 0, 0
    while i < len(a) or j < len(b):
        if j >= len(b) or (i < len(a) and i * len(b) <= j * len(a)):
            out.append(a[i]); i += 1
        else:
            out.append(b[j]); j += 1
    return out


@jax.jit
def pallas_gated_mix__compressed_kv_cla__gqa_block_cached__decode_kernel(
    A_x: jax.Array,
    A_c_kv: jax.Array,
    A_w_q: jax.Array,
    A_w_uk: jax.Array,
    A_w_uv: jax.Array,
    A_w_o: jax.Array,
    B_x: jax.Array,
    B_k_cache: jax.Array,
    B_v_cache: jax.Array,
    B_wq: jax.Array,
    B_wo: jax.Array,
    gate_w: jax.Array,
):
    B, Sq, M = A_x.shape
    _, Sk, Dc = A_c_kv.shape
    _, H, D = A_w_q.shape
    assert B == 1 and Sq == 1 and D == 128 and H == 32
    assert B_k_cache.shape == (1, H, Sk, D) and B_v_cache.shape == (1, H, Sk, D)
    HD = H * D
    scale = float(D) ** -0.5
    NXC = M // 128
    NCB = Dc // 128
    UH = 2 * Sk * D * 2 // PERIOD
    LOOK = -(-WLO // UH)
    NBUF = LOOK + 2
    assert sum(WO_GROUPS) == HD and DLT <= WLO and UH % HB == 0 and HB <= WLO - DLT
    H0 = 32 - HN

    w_q2 = A_w_q.reshape(M * H, D)
    w_uk2 = A_w_uk.reshape(Dc * H, D)
    w_uv2 = A_w_uv.reshape(Dc * H, D)
    w_o2 = A_w_o.reshape(HD, M)

    def kernel(x_hbm, gw_hbm, wqb_hbm, k_hbm, v_hbm, wqa_hbm, wuk_hbm, ckv_hbm,
               wuv_hbm, woa_hbm, wob_hbm,
               o_ref,
               x_v, gw_v, wqb_v, kbuf, vbuf, wqa_v, wuk_v, ckv_v, wuv_v, woa_v, wob_v,
               qb_s, ob_s,
               sem_w, sem_k, sem_v, sem_o, sem_b):
        def pair(sem, idx):
            return (sem.at[0, idx], sem.at[1, idx])

        cp_x = pltpu.make_async_copy(x_hbm, x_v, sem_w.at[0, 0])
        cp_gw = pltpu.make_async_copy(gw_hbm, gw_v, sem_w.at[1, 0])

        assert HD * 2 * 8 == PERIOD
        u_wqb = [_col_unit(wqb_hbm, wqb_v, pair(sem_w, 1), r, 8, HD, PHI['wqb'] * 64)
                 for r in range(0, M, 8)]
        u_wqa = _row_units(wqa_hbm, wqa_v, lambda r: pair(sem_w, 1), M * H, 2 * D, PHI['wqa'])
        u_wuk = _row_units(wuk_hbm, wuk_v, lambda r: pair(sem_w, 2), Dc * H, 2 * D, PHI['wuk'])
        u_wuv = _row_units(wuv_hbm, wuv_v, lambda r: pair(sem_w, 2), Dc * H, 2 * D, PHI['wuv'])
        u_ckv = _row_units(ckv_hbm.at[0], ckv_v, lambda r: pair(sem_w, 3), Sk, 2 * Dc, PHI['ckv'])
        u_p = _merge(u_wqb, u_wqa)
        u_t1 = _merge(u_wuk, u_wuv)
        u_t2 = _merge(u_ckv[:len(u_ckv) // 2], u_ckv[len(u_ckv) // 2:])
        wo_start = [sum(WO_GROUPS[:i]) for i in range(len(WO_GROUPS))]
        grp = lambda r: max(i for i, o in enumerate(wo_start) if o <= r)
        u_woa = _row_units(woa_hbm, woa_v, lambda r: pair(sem_o, grp(r)), HD, 2 * M, PHI['woa'])
        u_wob = _row_units(wob_hbm, wob_v, lambda r: pair(sem_o, grp(r)), HD, 2 * M, PHI['wob'])
        t3_groups = [_merge([u for u in u_woa if grp(u.row0) == gi], [u for u in u_wob if grp(u.row0) == gi])
                     for gi in range(len(WO_GROUPS))]
        u_t3 = [u for gr in t3_groups for u in gr]

        if 't1' in DROP: u_t1 = []
        if 't2' in DROP: u_t2 = []
        if 't3' in DROP: u_t3 = u_t3[-64:]
        if 'p' in DROP: u_p = u_p[:64]

        def head_units(h, slot):
            uk = _row_units(k_hbm.at[0, h], kbuf.at[slot], lambda r: pair(sem_k, slot), Sk, 2 * D, PHI['kv'])
            uv = _row_units(v_hbm.at[0, h], vbuf.at[slot], lambda r: pair(sem_v, slot), Sk, 2 * D, PHI['kv'])
            return [u for kv in zip(uk, uv) for u in kv]

        class Seq:
            def __init__(self, units, lim, early=0):
                self.u, self.lim, self.pos = units, lim, 0
                self.early = early

            def step(self, k):
                j = k - DLT
                if j < len(self.u) - self.early:
                    self.u[j].start_hi()
                if k < len(self.u):
                    self.u[k].start_lo()

            def adv(self, n):
                for i in range(self.pos, min(self.pos + n, self.lim)):
                    if i % HB == 0:
                        for k in range(i, min(i + HB, self.lim)):
                            self.u[k].wait_hi()
                    self.u[i].wait_lo()
                    self.step(i + WLO)
                    self.pos = i + 1

            def adv_to(self, target):
                self.adv(max(0, target - self.pos))

            def tick(self, n):
                self.adv(n * TICK // 4)

        static_heads = lambda lo, hi: [u for h in range(lo, hi) for u in head_units(h, h % NBUF)]
        npre = len(u_p)
        assert npre % HB == 0 and npre >= WLO
        pro = Seq(u_p + static_heads(H0, H0 + LOOK + 1), npre + UH)
        early = DLT if WRAP else 0
        end = Seq(static_heads(H - LOOK, H) + u_t1 + u_t2 + u_t3, 0, early)
        end.lim = len(end.u)

        cp_x.start(priority=PQ0)
        cp_gw.start(priority=PQ0)
        if BARRIER:
            pl.semaphore_signal(sem_b, WLO)
        for k in range(WLO):
            if BARRIER:
                pl.semaphore_wait(sem_b, 1)
            if k < DLT:
                if WRAP:
                    end.u[len(end.u) - DLT + k].start_hi()
            else:
                pro.u[k - DLT].start_hi()
            pro.u[k].start_lo()

        cp_x.wait()
        cp_gw.wait()
        x = x_v[0].astype(_F32)
        gw = gw_v[...].astype(_F32).reshape(1, M)
        g = jax.nn.sigmoid(jnp.sum(x * gw, axis=-1, keepdims=True))
        x8 = jnp.broadcast_to(x, (8, M)).astype(_BF16)

        pro.adv_to(npre)
        QB = HD // 4
        for c in range(4):
            qb = _dot(x8, wqb_v[:, pl.ds(c * QB, QB)]) * scale
            for h in range(QB // D):
                qb_s[c * (QB // D) + h] = qb[:, h * D:(h + 1) * D]
            pro.tick(4)

        def attend(h, slot, seq):
            stop = seq.pos + UH
            if SKIP_COMPUTE:
                ob_s[h] = qb_s[h]
                seq.adv_to(stop)
                return
            HS = Sk // 2
            q = qb_s[h].astype(_BF16)
            seq.adv(SPLITS[0])
            s0 = _dot_nt(q, kbuf[slot, pl.ds(0, HS), :])
            seq.adv(SPLITS[1])
            s1 = _dot_nt(q, kbuf[slot, pl.ds(HS, HS), :])
            seq.adv(SPLITS[2])
            m = jnp.maximum(jnp.max(s0, axis=-1, keepdims=True), jnp.max(s1, axis=-1, keepdims=True))
            p0 = jnp.exp(s0 - m)
            p1 = jnp.exp(s1 - m)
            l = jnp.sum(p0, axis=-1, keepdims=True) + jnp.sum(p1, axis=-1, keepdims=True)
            p0 = p0.astype(_BF16)
            p1 = p1.astype(_BF16)
            seq.adv(SPLITS[3])
            o = _dot(p0, vbuf[slot, pl.ds(0, HS), :])
            seq.adv(SPLITS[4])
            o = o + _dot(p1, vbuf[slot, pl.ds(HS, HS), :])
            ob_s[h] = o / l
            seq.adv_to(stop)

        pro.adv_to(pro.lim)

        def body(h, carry):
            units = []
            for k in range(1, LOOK + 2):
                units = units + head_units(h + k, lax.rem(h + k, NBUF))
            attend(h, lax.rem(h, NBUF), Seq(units, UH))
            return carry

        lax.fori_loop(H0, H - LOOK - 1, body, 0)

        for h in range(H - LOOK - 1, H):
            attend(h, h % NBUF, end)
        p_t1 = LOOK * UH + len(u_t1)
        p_t2 = p_t1 + len(u_t2)

        if SKIP_A:
            end.adv_to(end.lim)
            o_ref[0] = (x * g + ob_s[31][0:1, 0:1]).astype(o_ref.dtype)
            return

        e_row = lax.broadcasted_iota(jnp.int32, (128, HD), 0)
        e_col = lax.broadcasted_iota(jnp.int32, (128, HD), 1)
        e0 = jnp.where(e_row == (e_col >> 5), 1.0, 0.0).astype(_BF16)
        d_row = lax.broadcasted_iota(jnp.int32, (H, HD), 0)
        d_col = lax.broadcasted_iota(jnp.int32, (H, HD), 1)
        diag = (d_col & (H - 1)) == d_row
        x5 = jnp.concatenate(
            [x[:, c * 128:(c + 1) * 128] for c in range(NXC)]
            + [jnp.zeros((8 - NXC, 128), _F32)], axis=0).astype(_BF16)
        xr = _dot(x5, e0)
        end.tick(4)
        qa = jnp.zeros((H, D), _F32)
        for c in range(NXC):
            sc = jnp.where(diag, jnp.broadcast_to(xr[c:c + 1, :], (H, HD)), 0.0).astype(_BF16)
            qa = qa + _dot(sc, wqa_v[pl.ds(c * HD, HD), :])
            end.tick(3)
        qa = (qa * scale).astype(_BF16)

        end.adv_to(p_t1)
        qabs = []
        for b in range(NCB):
            t = _dot_nt(qa, wuk_v[pl.ds(b * HD, HD), :])
            mb = jnp.where(diag, t, 0.0).astype(_BF16)
            end.tick(4)
            qabs.append(_dot_nt(mb, e0))
            end.tick(4)
        qabs = jnp.concatenate(qabs, axis=1).astype(_BF16)

        end.adv_to(p_t2)
        KB = Sk // 4
        s = []
        for kb in range(4):
            s.append(_dot_nt(qabs, ckv_v[pl.ds(kb * KB, KB), :]))
            end.tick(3)
        s = jnp.concatenate(s, axis=1)
        m = jnp.max(s, axis=-1, keepdims=True)
        p = jnp.exp(s - m)
        l = jnp.sum(p, axis=-1, keepdims=True)
        p = p.astype(_BF16)
        end.tick(3)
        cl = jnp.zeros((H, Dc), _F32)
        for kb in range(4):
            cl = cl + _dot(p[:, kb * KB:(kb + 1) * KB], ckv_v[pl.ds(kb * KB, KB), :])
            end.tick(3)
        cl = (cl / l).astype(_BF16)

        ctx = jnp.zeros((H, D), _F32)
        for b in range(NCB):
            xb = _dot(cl[:, b * 128:(b + 1) * 128], e0)
            sb = jnp.where(diag, xb, 0.0).astype(_BF16)
            ctx = ctx + _dot(sb, wuv_v[pl.ds(b * HD, HD), :])
            end.tick(4)

        sub = lax.broadcasted_iota(jnp.int32, (8, D), 0)
        ctx_flat = jnp.concatenate(
            [jnp.where(sub == (h % 8), ctx[8 * (h // 8):8 * (h // 8) + 8, :], 0.0) for h in range(H)],
            axis=1).astype(_BF16)
        o_flat = jnp.concatenate([ob_s[h] for h in range(H)], axis=1).astype(_BF16)
        one_g = 1.0 - g

        acc_a = jnp.zeros((8, M), _F32)
        acc_b = jnp.zeros((8, M), _F32)
        o = 0
        target = p_t2
        for n, gr in zip(WO_GROUPS, t3_groups):
            target += len(gr)
            end.adv_to(target)
            acc_a = acc_a + _dot(ctx_flat[:, o:o + n], woa_v[pl.ds(o, n), :])
            acc_b = acc_b + _dot(o_flat[:, o:o + n], wob_v[pl.ds(o, n), :])
            o += n
        assert end.pos == end.lim
        a = jnp.sum(acc_a, axis=0, keepdims=True)
        o_ref[0] = (g * a + one_g * acc_b[0:1, :]).astype(o_ref.dtype)

    any_spec = pl.BlockSpec(memory_space=pl.ANY)
    scratch = [
        pltpu.VMEM((1, 1, M), _BF16),
        pltpu.VMEM((M,), _BF16),
        pltpu.VMEM((M, HD), _BF16),
        pltpu.VMEM((NBUF, Sk, D), _BF16),
        pltpu.VMEM((NBUF, Sk, D), _BF16),
        pltpu.VMEM((M * H, D), _BF16),
        pltpu.VMEM((Dc * H, D), _BF16),
        pltpu.VMEM((Sk, Dc), _BF16),
        pltpu.VMEM((Dc * H, D), _BF16),
        pltpu.VMEM((HD, M), _BF16),
        pltpu.VMEM((HD, M), _BF16),
        pltpu.VMEM((H, 8, D), _F32),
        pltpu.VMEM((H, 8, D), _F32),
        pltpu.SemaphoreType.DMA((2, 4)),
        pltpu.SemaphoreType.DMA((2, NBUF)),
        pltpu.SemaphoreType.DMA((2, NBUF)),
        pltpu.SemaphoreType.DMA((2, len(WO_GROUPS))),
        pltpu.SemaphoreType.REGULAR,
    ]
    return pl.pallas_call(
        kernel,
        out_shape=jax.ShapeDtypeStruct((B, Sq, M), A_x.dtype),
        in_specs=[any_spec] * 11,
        out_specs=pl.BlockSpec(memory_space=pltpu.VMEM),
        scratch_shapes=scratch,
        compiler_params=pltpu.CompilerParams(
            vmem_limit_bytes=100 * 1024 * 1024,
            disable_semaphore_checks=NOSEM, disable_bounds_checks=NOBND),
    )(A_x, gate_w, B_wq, B_k_cache, B_v_cache, w_q2, w_uk2, A_c_kv, w_uv2, w_o2, B_wo)
```

```python
import jax
import jax.numpy as jnp
from jax import lax
import jax.experimental.pallas as pl
import jax.experimental.pallas.tpu as pltpu

_NT = (((1,), (1,)), ((), ()))
_F32 = jnp.float32
_BF16 = jnp.bfloat16

PERIOD = 64 * 1024
PHI = dict(kv=30, wqb=30, wqa=28, wuk=28, ckv=24, wuv=28, woa=30, wob=30)
WLO = 56
DLT = 24
TICK = 6
HB = 8
SPLITS = (6, 6, 6, 6, 6)
WO_GROUPS = (1024, 1024, 1024, 512, 256, 128, 128)
NPACED = 3
PQ_HI, PQ_LO = 0, 1


def _dot(a, b):
    return jnp.dot(a, b, preferred_element_type=_F32)


def _dot_nt(a, b):
    return lax.dot_general(a, b, _NT, preferred_element_type=_F32)


class _Unit:
    def __init__(self, hi, lo):
        self.hi, self.lo = hi, lo

    def start_hi(self):
        if self.hi is not None:
            self.hi().start(priority=PQ_HI)

    def start_lo(self):
        self.lo().start(priority=PQ_LO)

    def wait_hi(self):
        if self.hi is not None:
            self.hi().wait()

    def wait_lo(self):
        self.lo().wait()


def _row_units(src, dst, sems_of_row, nrows, row_bytes, phi_kib):
    tb = 8 * row_bytes
    near = lambda off: min(nrows, 8 * ((off + tb // 2) // tb))
    out = []
    k = 0
    while near(k * PERIOD) < nrows:
        a, m, b = near(k * PERIOD), near(k * PERIOD + phi_kib * 1024), near((k + 1) * PERIOD)
        sems = sems_of_row(a)
        mk = lambda r, n, q, sems=sems: (lambda: pltpu.make_async_copy(
            src.at[pl.ds(r, n)], dst.at[pl.ds(r, n)], sems[q]))
        if m >= b or m <= a:
            u = _Unit(None, mk(a, b - a, 1))
        else:
            u = _Unit(mk(a, m - a, 0), mk(m, b - m, 1))
        u.row0, u.row1 = a, b
        out.append(u)
        k += 1
    return out


def _col_unit(src, dst, sems, r0, n, ncols, ch):
    mk = lambda a, k, q: (lambda: pltpu.make_async_copy(
        src.at[pl.ds(r0, n), pl.ds(a, k)], dst.at[pl.ds(r0, n), pl.ds(a, k)], sems[q]))
    return _Unit(mk(0, ch, 0), mk(ch, ncols - ch, 1))


def _merge(a, b):
    out, i, j = [], 0, 0
    while i < len(a) or j < len(b):
        if j >= len(b) or (i < len(a) and i * len(b) <= j * len(a)):
            out.append(a[i])
            i += 1
        else:
            out.append(b[j])
            j += 1
    return out


class _Stream:
    def __init__(self, units, lim, last=False):
        self.u, self.lim, self.pos, self.last = units, lim, 0, last

    def step(self, k):
        if k - DLT < len(self.u):
            self.u[k - DLT].start_hi()
        if k < len(self.u):
            self.u[k].start_lo()

    def adv(self, n):
        for i in range(self.pos, min(self.pos + n, self.lim)):
            if i % HB == 0:
                for k in range(i, min(i + HB, self.lim)):
                    self.u[k].wait_hi()
            self.u[i].wait_lo()
            self.step(i + WLO)
            if self.last and i == self.lim - 1:
                for k in range(i + 1 + WLO, len(self.u) + DLT):
                    self.step(k)
            self.pos = i + 1

    def adv_to(self, target):
        self.adv(max(0, target - self.pos))

    def tick(self, n):
        self.adv(n * TICK // 4)


@jax.jit
def pallas_gated_mix__compressed_kv_cla__gqa_block_cached__decode_kernel(
    A_x: jax.Array,
    A_c_kv: jax.Array,
    A_w_q: jax.Array,
    A_w_uk: jax.Array,
    A_w_uv: jax.Array,
    A_w_o: jax.Array,
    B_x: jax.Array,
    B_k_cache: jax.Array,
    B_v_cache: jax.Array,
    B_wq: jax.Array,
    B_wo: jax.Array,
    gate_w: jax.Array,
):
    del B_x
    B, Sq, M = A_x.shape
    _, Sk, Dc = A_c_kv.shape
    _, H, D = A_w_q.shape
    assert B == 1 and Sq == 1 and D == 128 and H == 32
    assert B_k_cache.shape == (1, H, Sk, D) and B_v_cache.shape == (1, H, Sk, D)
    HD = H * D
    scale = float(D) ** -0.5
    NXC = M // 128
    NCB = Dc // 128
    UH = 2 * Sk * D * 2 // PERIOD
    LOOK = -(-WLO // UH)
    NBUF = LOOK + 2
    NEXACT = len(WO_GROUPS) - NPACED
    assert sum(WO_GROUPS) == HD and UH % HB == 0 and HB <= WLO - DLT and sum(SPLITS) <= UH
    assert HD * 2 * 8 == PERIOD and M % 128 == 0 and M // 128 <= 8

    w_q2 = A_w_q.reshape(M * H, D)
    w_uk2 = A_w_uk.reshape(Dc * H, D)
    w_uv2 = A_w_uv.reshape(Dc * H, D)
    w_o2 = A_w_o.reshape(HD, M)

    def kernel(x_hbm, gw_hbm, wqb_hbm, k_hbm, v_hbm, wqa_hbm, wuk_hbm, ckv_hbm,
               wuv_hbm, woa_hbm, wob_hbm,
               o_ref,
               x_v, gw_v, wqb_v, kbuf, vbuf, wqa_v, wuk_v, ckv_v, wuv_v, woa_v, wob_v,
               qb_s, ob_s,
               sem_w, sem_k, sem_v, sem_o, sem_f):
        def pair(sem, idx):
            return (sem.at[0, idx], sem.at[1, idx])

        cp_x = pltpu.make_async_copy(x_hbm, x_v, sem_w.at[0, 0])
        cp_gw = pltpu.make_async_copy(gw_hbm, gw_v, sem_w.at[1, 0])

        u_wqb = [_col_unit(wqb_hbm, wqb_v, pair(sem_w, 1), r, 8, HD, PHI['wqb'] * 64)
                 for r in range(0, M, 8)]
        u_wqa = _row_units(wqa_hbm, wqa_v, lambda r: pair(sem_w, 1), M * H, 2 * D, PHI['wqa'])
        u_wuk = _row_units(wuk_hbm, wuk_v, lambda r: pair(sem_w, 2), Dc * H, 2 * D, PHI['wuk'])
        u_wuv = _row_units(wuv_hbm, wuv_v, lambda r: pair(sem_w, 2), Dc * H, 2 * D, PHI['wuv'])
        u_ckv = _row_units(ckv_hbm.at[0], ckv_v, lambda r: pair(sem_w, 3), Sk, 2 * Dc, PHI['ckv'])
        u_pre = _merge(u_wqb, u_wqa)
        u_up = _merge(u_wuk, u_wuv)
        u_lat = _merge(u_ckv[:len(u_ckv) // 2], u_ckv[len(u_ckv) // 2:])

        wo_start = [sum(WO_GROUPS[:i]) for i in range(len(WO_GROUPS))]
        grp = lambda r: max(i for i, o in enumerate(wo_start) if o <= r)

        def wo_sems(which):
            def f(r):
                gi = grp(r)
                if gi < NPACED:
                    return pair(sem_o, gi)
                return (sem_f.at[which, gi - NPACED],) * 2
            return f

        u_woa = _row_units(woa_hbm, woa_v, wo_sems(0), HD, 2 * M, PHI['woa'])
        u_wob = _row_units(wob_hbm, wob_v, wo_sems(1), HD, 2 * M, PHI['wob'])
        in_grp = lambda us, gi: [u for u in us if grp(u.row0) == gi]
        wo_groups = [_merge(in_grp(u_woa, gi), in_grp(u_wob, gi)) for gi in range(len(WO_GROUPS))]
        u_out = [u for gr in wo_groups for u in gr]

        def head_units(h, slot):
            uk = _row_units(k_hbm.at[0, h], kbuf.at[slot], lambda r: pair(sem_k, slot), Sk, 2 * D, PHI['kv'])
            uv = _row_units(v_hbm.at[0, h], vbuf.at[slot], lambda r: pair(sem_v, slot), Sk, 2 * D, PHI['kv'])
            return [u for kv in zip(uk, uv) for u in kv]

        static_heads = lambda lo, hi: [u for h in range(lo, hi) for u in head_units(h, h % NBUF)]
        npre = len(u_pre)
        assert npre % HB == 0 and npre >= WLO
        pro = _Stream(u_pre + static_heads(0, LOOK + 1), npre + UH)
        end_units = static_heads(H - LOOK, H) + u_up + u_lat + u_out
        nexact = sum(len(gr) for gr in wo_groups[NPACED:])
        assert nexact <= WLO
        end = _Stream(end_units, len(end_units) - nexact, last=True)

        cp_x.start(priority=PQ_HI)
        cp_gw.start(priority=PQ_HI)
        for k in range(WLO):
            if k >= DLT:
                pro.u[k - DLT].start_hi()
            pro.u[k].start_lo()

        cp_x.wait()
        cp_gw.wait()
        x = x_v[0].astype(_F32)
        gw = gw_v[...].astype(_F32).reshape(1, M)
        g = jax.nn.sigmoid(jnp.sum(x * gw, axis=-1, keepdims=True))
        x8 = jnp.broadcast_to(x, (8, M)).astype(_BF16)

        pro.adv_to(npre)
        QB = HD // 4
        for c in range(4):
            qb = _dot(x8, wqb_v[:, pl.ds(c * QB, QB)]) * scale
            for h in range(QB // D):
                qb_s[c * (QB // D) + h] = qb[:, h * D:(h + 1) * D]
            pro.tick(4)
        pro.adv_to(pro.lim)

        def attend(h, slot, seq):
            stop = seq.pos + UH
            HS = Sk // 2
            q = qb_s[h].astype(_BF16)
            seq.adv(SPLITS[0])
            s0 = _dot_nt(q, kbuf[slot, pl.ds(0, HS), :])
            seq.adv(SPLITS[1])
            s1 = _dot_nt(q, kbuf[slot, pl.ds(HS, HS), :])
            seq.adv(SPLITS[2])
            m = jnp.maximum(jnp.max(s0, axis=-1, keepdims=True), jnp.max(s1, axis=-1, keepdims=True))
            p0 = jnp.exp(s0 - m)
            p1 = jnp.exp(s1 - m)
            l = jnp.sum(p0, axis=-1, keepdims=True) + jnp.sum(p1, axis=-1, keepdims=True)
            p0 = p0.astype(_BF16)
            p1 = p1.astype(_BF16)
            seq.adv(SPLITS[3])
            o = _dot(p0, vbuf[slot, pl.ds(0, HS), :])
            seq.adv(SPLITS[4])
            o = o + _dot(p1, vbuf[slot, pl.ds(HS, HS), :])
            ob_s[h] = o / l
            seq.adv_to(stop)

        def body(h, carry):
            units = []
            for k in range(1, LOOK + 2):
                units = units + head_units(h + k, lax.rem(h + k, NBUF))
            attend(h, lax.rem(h, NBUF), _Stream(units, UH))
            return carry

        lax.fori_loop(0, H - LOOK - 1, body, 0)
        for h in range(H - LOOK - 1, H):
            attend(h, h % NBUF, end)

        p_up = LOOK * UH + len(u_up)
        p_lat = p_up + len(u_lat)
        e_row = lax.broadcasted_iota(jnp.int32, (128, HD), 0)
        e_col = lax.broadcasted_iota(jnp.int32, (128, HD), 1)
        e0 = jnp.where(e_row == (e_col >> 5), 1.0, 0.0).astype(_BF16)
        d_row = lax.broadcasted_iota(jnp.int32, (H, HD), 0)
        d_col = lax.broadcasted_iota(jnp.int32, (H, HD), 1)
        diag = (d_col & (H - 1)) == d_row
        x5 = jnp.concatenate(
            [x[:, c * 128:(c + 1) * 128] for c in range(NXC)]
            + [jnp.zeros((8 - NXC, 128), _F32)], axis=0).astype(_BF16)
        xr = _dot(x5, e0)
        end.tick(4)
        qa = jnp.zeros((H, D), _F32)
        for c in range(NXC):
            sc = jnp.where(diag, jnp.broadcast_to(xr[c:c + 1, :], (H, HD)), 0.0).astype(_BF16)
            qa = qa + _dot(sc, wqa_v[pl.ds(c * HD, HD), :])
            end.tick(3)
        qa = (qa * scale).astype(_BF16)

        end.adv_to(p_up)
        qabs = []
        for b in range(NCB):
            t = _dot_nt(qa, wuk_v[pl.ds(b * HD, HD), :])
            mb = jnp.where(diag, t, 0.0).astype(_BF16)
            end.tick(4)
            qabs.append(_dot_nt(mb, e0))
            end.tick(4)
        qabs = jnp.concatenate(qabs, axis=1).astype(_BF16)

        end.adv_to(p_lat)
        KB = Sk // 4
        s = []
        for kb in range(4):
            s.append(_dot_nt(qabs, ckv_v[pl.ds(kb * KB, KB), :]))
            end.tick(3)
        s = jnp.concatenate(s, axis=1)
        m = jnp.max(s, axis=-1, keepdims=True)
        p = jnp.exp(s - m)
        l = jnp.sum(p, axis=-1, keepdims=True)
        p = p.astype(_BF16)
        end.tick(3)
        cl = jnp.zeros((H, Dc), _F32)
        for kb in range(4):
            cl = cl + _dot(p[:, kb * KB:(kb + 1) * KB], ckv_v[pl.ds(kb * KB, KB), :])
            end.tick(3)
        cl = (cl / l).astype(_BF16)

        ctx = jnp.zeros((H, D), _F32)
        for b in range(NCB):
            xb = _dot(cl[:, b * 128:(b + 1) * 128], e0)
            sb = jnp.where(diag, xb, 0.0).astype(_BF16)
            ctx = ctx + _dot(sb, wuv_v[pl.ds(b * HD, HD), :])
            end.tick(4)

        sub = lax.broadcasted_iota(jnp.int32, (8, D), 0)
        ctx = ctx * g
        lhs_a = jnp.concatenate(
            [jnp.where(sub == (h % 8), ctx[8 * (h // 8):8 * (h // 8) + 8, :], 0.0) for h in range(H)],
            axis=1).astype(_BF16)
        one_g = 1.0 - g
        lhs_b = jnp.concatenate(
            [jnp.where(sub == (h % 8), ob_s[h] * one_g, 0.0) for h in range(H)],
            axis=1).astype(_BF16)

        acc = jnp.zeros((8, M), _F32)
        o = 0
        target = p_lat
        for gi, (n, gr) in enumerate(zip(WO_GROUPS, wo_groups)):
            if gi < NPACED:
                target += len(gr)
                end.adv_to(target)
            else:
                for which, (us, buf) in enumerate(((u_woa, woa_v), (u_wob, wob_v))):
                    mine = in_grp(us, gi)
                    rows = buf.at[pl.ds(mine[0].row0, mine[-1].row1 - mine[0].row0)]
                    pltpu.make_async_copy(rows, rows, sem_f.at[which, gi - NPACED]).wait()
            acc = acc + _dot(lhs_a[:, o:o + n], woa_v[pl.ds(o, n), :])
            acc = acc + _dot(lhs_b[:, o:o + n], wob_v[pl.ds(o, n), :])
            o += n
        assert end.pos == end.lim
        o_ref[0] = jnp.sum(acc, axis=0, keepdims=True).astype(o_ref.dtype)

    any_spec = pl.BlockSpec(memory_space=pl.ANY)
    scratch = [
        pltpu.VMEM((1, 1, M), _BF16),
        pltpu.VMEM((M,), _BF16),
        pltpu.VMEM((M, HD), _BF16),
        pltpu.VMEM((NBUF, Sk, D), _BF16),
        pltpu.VMEM((NBUF, Sk, D), _BF16),
        pltpu.VMEM((M * H, D), _BF16),
        pltpu.VMEM((Dc * H, D), _BF16),
        pltpu.VMEM((Sk, Dc), _BF16),
        pltpu.VMEM((Dc * H, D), _BF16),
        pltpu.VMEM((HD, M), _BF16),
        pltpu.VMEM((HD, M), _BF16),
        pltpu.VMEM((H, 8, D), _F32),
        pltpu.VMEM((H, 8, D), _F32),
        pltpu.SemaphoreType.DMA((2, 4)),
        pltpu.SemaphoreType.DMA((2, NBUF)),
        pltpu.SemaphoreType.DMA((2, NBUF)),
        pltpu.SemaphoreType.DMA((2, NPACED)),
        pltpu.SemaphoreType.DMA((2, NEXACT)),
    ]
    return pl.pallas_call(
        kernel,
        out_shape=jax.ShapeDtypeStruct((B, Sq, M), A_x.dtype),
        in_specs=[any_spec] * 11,
        out_specs=pl.BlockSpec(memory_space=pltpu.VMEM),
        scratch_shapes=scratch,
        compiler_params=pltpu.CompilerParams(
            vmem_limit_bytes=100 * 1024 * 1024,
            disable_semaphore_checks=True, disable_bounds_checks=True),
    )(A_x, gate_w, B_wq, B_k_cache, B_v_cache, w_q2, w_uk2, A_c_kv, w_uv2, w_o2, B_wo)
```

```python
import jax
import jax.numpy as jnp
from jax import lax
import jax.experimental.pallas as pl
import jax.experimental.pallas.tpu as pltpu

_NT = (((1,), (1,)), ((), ()))
_F32 = jnp.float32
_BF16 = jnp.bfloat16

PERIOD = 64 * 1024
PHI = dict(kv=30, wqb=30, wqa=28, wuk=28, ckv=24, wuv=28, woa=30, wob=30)
OFF = 18
WLO = 56
DLT = 24
TICK = 6
HB = 8
SPLITS = (6, 6, 6, 6, 6)
WO_GROUPS = (1024, 1024, 1024, 512, 256, 128, 128)
NPACED = 3
PQ_HI, PQ_LO = 0, 1


def _dot(a, b):
    return jnp.dot(a, b, preferred_element_type=_F32)


def _dot_nt(a, b):
    return lax.dot_general(a, b, _NT, preferred_element_type=_F32)


class _Unit:
    def __init__(self, hi, lo):
        self.hi, self.lo = hi, lo

    def start_hi(self):
        if self.hi is not None:
            self.hi().start(priority=PQ_HI)

    def start_lo(self):
        self.lo().start(priority=PQ_LO)

    def wait_hi(self):
        if self.hi is not None:
            self.hi().wait()

    def wait_lo(self):
        self.lo().wait()


def _row_units(src, dst, sems_of_row, nrows, row_bytes, phi_kib):
    tb = 8 * row_bytes
    near = lambda off: min(nrows, 8 * ((off + tb // 2) // tb))
    out = []
    k = 0
    cut = lambda k: 0 if k == 0 else (nrows if k * PERIOD >= nrows * row_bytes else near(k * PERIOD + OFF * 1024))
    while cut(k) < nrows:
        a, m, b = cut(k), near(k * PERIOD + phi_kib * 1024), cut(k + 1)
        sems = sems_of_row(a)
        mk = lambda r, n, q, sems=sems: (lambda: pltpu.make_async_copy(
            src.at[pl.ds(r, n)], dst.at[pl.ds(r, n)], sems[q]))
        if m >= b or m <= a:
            u = _Unit(None, mk(a, b - a, 1))
        else:
            u = _Unit(mk(a, m - a, 0), mk(m, b - m, 1))
        u.row0, u.row1 = a, b
        out.append(u)
        k += 1
    return out


def _col_unit(src, dst, sems, r0, n, ncols, ch):
    mk = lambda a, k, q: (lambda: pltpu.make_async_copy(
        src.at[pl.ds(r0, n), pl.ds(a, k)], dst.at[pl.ds(r0, n), pl.ds(a, k)], sems[q]))
    return _Unit(mk(0, ch, 0), mk(ch, ncols - ch, 1))


def _merge(a, b):
    out, i, j = [], 0, 0
    while i < len(a) or j < len(b):
        if j >= len(b) or (i < len(a) and i * len(b) <= j * len(a)):
            out.append(a[i])
            i += 1
        else:
            out.append(b[j])
            j += 1
    return out


class _Stream:
    def __init__(self, units, lim, last=False):
        self.u, self.lim, self.pos, self.last = units, lim, 0, last

    def step(self, k):
        if k - DLT < len(self.u):
            self.u[k - DLT].start_hi()
        if k < len(self.u):
            self.u[k].start_lo()

    def adv(self, n):
        for i in range(self.pos, min(self.pos + n, self.lim)):
            if i % HB == 0:
                for k in range(i, min(i + HB, self.lim)):
                    self.u[k].wait_hi()
            self.u[i].wait_lo()
            self.step(i + WLO)
            if self.last and i == self.lim - 1:
                for k in range(i + 1 + WLO, len(self.u) + DLT):
                    self.step(k)
            self.pos = i + 1

    def adv_to(self, target):
        self.adv(max(0, target - self.pos))

    def tick(self, n):
        self.adv(n * TICK // 4)


@jax.jit
def pallas_gated_mix__compressed_kv_cla__gqa_block_cached__decode_kernel(
    A_x: jax.Array,
    A_c_kv: jax.Array,
    A_w_q: jax.Array,
    A_w_uk: jax.Array,
    A_w_uv: jax.Array,
    A_w_o: jax.Array,
    B_x: jax.Array,
    B_k_cache: jax.Array,
    B_v_cache: jax.Array,
    B_wq: jax.Array,
    B_wo: jax.Array,
    gate_w: jax.Array,
):
    del B_x
    B, Sq, M = A_x.shape
    _, Sk, Dc = A_c_kv.shape
    _, H, D = A_w_q.shape
    assert B == 1 and Sq == 1 and D == 128 and H == 32
    assert B_k_cache.shape == (1, H, Sk, D) and B_v_cache.shape == (1, H, Sk, D)
    HD = H * D
    scale = float(D) ** -0.5
    NXC = M // 128
    NCB = Dc // 128
    UH = 2 * Sk * D * 2 // PERIOD
    LOOK = -(-WLO // UH)
    NBUF = LOOK + 2
    NEXACT = len(WO_GROUPS) - NPACED
    assert sum(WO_GROUPS) == HD and UH % HB == 0 and HB <= WLO - DLT and sum(SPLITS) <= UH
    assert HD * 2 * 8 == PERIOD and M % 128 == 0 and M // 128 <= 8

    w_q2 = A_w_q.reshape(M * H, D)
    w_uk2 = A_w_uk.reshape(Dc * H, D)
    w_uv2 = A_w_uv.reshape(Dc * H, D)
    w_o2 = A_w_o.reshape(HD, M)

    def kernel(x_hbm, gw_hbm, wqb_hbm, k_hbm, v_hbm, wqa_hbm, wuk_hbm, ckv_hbm,
               wuv_hbm, woa_hbm, wob_hbm,
               o_ref,
               x_v, gw_v, wqb_v, kbuf, vbuf, wqa_v, wuk_v, ckv_v, wuv_v, woa_v, wob_v,
               qb_s, ob_s,
               sem_w, sem_k, sem_v, sem_o, sem_f):
        def pair(sem, idx):
            return (sem.at[0, idx], sem.at[1, idx])

        cp_x = pltpu.make_async_copy(x_hbm, x_v, sem_w.at[0, 0])
        cp_gw = pltpu.make_async_copy(gw_hbm, gw_v, sem_w.at[1, 0])

        u_wqb = [_col_unit(wqb_hbm, wqb_v, pair(sem_w, 1), r, 8, HD, PHI['wqb'] * 64)
                 for r in range(0, M, 8)]
        u_wqa = _row_units(wqa_hbm, wqa_v, lambda r: pair(sem_w, 1), M * H, 2 * D, PHI['wqa'])
        u_wuk = _row_units(wuk_hbm, wuk_v, lambda r: pair(sem_w, 2), Dc * H, 2 * D, PHI['wuk'])
        u_wuv = _row_units(wuv_hbm, wuv_v, lambda r: pair(sem_w, 2), Dc * H, 2 * D, PHI['wuv'])
        u_ckv = _row_units(ckv_hbm.at[0], ckv_v, lambda r: pair(sem_w, 3), Sk, 2 * Dc, PHI['ckv'])
        u_pre = _merge(u_wqb, u_wqa)
        u_up = _merge(u_wuk, u_wuv)
        u_lat = _merge(u_ckv[:len(u_ckv) // 2], u_ckv[len(u_ckv) // 2:])

        wo_start = [sum(WO_GROUPS[:i]) for i in range(len(WO_GROUPS))]
        grp = lambda r: max(i for i, o in enumerate(wo_start) if o <= r)

        def wo_sems(which):
            def f(r):
                gi = grp(r)
                if gi < NPACED:
                    return pair(sem_o, gi)
                return (sem_f.at[which, gi - NPACED],) * 2
            return f

        u_woa = _row_units(woa_hbm, woa_v, wo_sems(0), HD, 2 * M, PHI['woa'])
        u_wob = _row_units(wob_hbm, wob_v, wo_sems(1), HD, 2 * M, PHI['wob'])
        in_grp = lambda us, gi: [u for u in us if grp(u.row0) == gi]
        wo_groups = [_merge(in_grp(u_woa, gi), in_grp(u_wob, gi)) for gi in range(len(WO_GROUPS))]
        u_out = [u for gr in wo_groups for u in gr]

        def head_units(h, slot):
            uk = _row_units(k_hbm.at[0, h], kbuf.at[slot], lambda r: pair(sem_k, slot), Sk, 2 * D, PHI['kv'])
            uv = _row_units(v_hbm.at[0, h], vbuf.at[slot], lambda r: pair(sem_v, slot), Sk, 2 * D, PHI['kv'])
            return [u for kv in zip(uk, uv) for u in kv]

        static_heads = lambda lo, hi: [u for h in range(lo, hi) for u in head_units(h, h % NBUF)]
        npre = len(u_pre)
        assert npre % HB == 0 and npre >= WLO
        pro = _Stream(u_pre + static_heads(0, LOOK + 1), npre + UH)
        end_units = static_heads(H - LOOK, H) + u_up + u_lat + u_out
        nexact = sum(len(gr) for gr in wo_groups[NPACED:])
        assert nexact <= WLO
        end = _Stream(end_units, len(end_units) - nexact, last=True)

        cp_x.start(priority=PQ_HI)
        cp_gw.start(priority=PQ_HI)
        for k in range(WLO):
            if k >= DLT:
                pro.u[k - DLT].start_hi()
            pro.u[k].start_lo()

        cp_x.wait()
        cp_gw.wait()
        x = x_v[0].astype(_F32)
        gw = gw_v[...].astype(_F32).reshape(1, M)
        g = jax.nn.sigmoid(jnp.sum(x * gw, axis=-1, keepdims=True))
        x8 = jnp.broadcast_to(x, (8, M)).astype(_BF16)

        pro.adv_to(npre)
        QB = HD // 4
        for c in range(4):
            qb = _dot(x8, wqb_v[:, pl.ds(c * QB, QB)]) * scale
            for h in range(QB // D):
                qb_s[c * (QB // D) + h] = qb[:, h * D:(h + 1) * D]
            pro.tick(4)
        pro.adv_to(pro.lim)

        def attend(h, slot, seq):
            stop = seq.pos + UH
            HS = Sk // 2
            q = qb_s[h].astype(_BF16)
            seq.adv(SPLITS[0])
            s0 = _dot_nt(q, kbuf[slot, pl.ds(0, HS), :])
            seq.adv(SPLITS[1])
            s1 = _dot_nt(q, kbuf[slot, pl.ds(HS, HS), :])
            seq.adv(SPLITS[2])
            m = jnp.maximum(jnp.max(s0, axis=-1, keepdims=True), jnp.max(s1, axis=-1, keepdims=True))
            p0 = jnp.exp(s0 - m)
            p1 = jnp.exp(s1 - m)
            l = jnp.sum(p0, axis=-1, keepdims=True) + jnp.sum(p1, axis=-1, keepdims=True)
            p0 = p0.astype(_BF16)
            p1 = p1.astype(_BF16)
            seq.adv(SPLITS[3])
            o = _dot(p0, vbuf[slot, pl.ds(0, HS), :])
            seq.adv(SPLITS[4])
            o = o + _dot(p1, vbuf[slot, pl.ds(HS, HS), :])
            ob_s[h] = o / l
            seq.adv_to(stop)

        def body(h, carry):
            units = []
            for k in range(1, LOOK + 2):
                units = units + head_units(h + k, lax.rem(h + k, NBUF))
            attend(h, lax.rem(h, NBUF), _Stream(units, UH))
            return carry

        lax.fori_loop(0, H - LOOK - 1, body, 0)
        for h in range(H - LOOK - 1, H):
            attend(h, h % NBUF, end)

        p_up = LOOK * UH + len(u_up)
        p_lat = p_up + len(u_lat)
        e_row = lax.broadcasted_iota(jnp.int32, (128, HD), 0)
        e_col = lax.broadcasted_iota(jnp.int32, (128, HD), 1)
        e0 = jnp.where(e_row == (e_col >> 5), 1.0, 0.0).astype(_BF16)
        d_row = lax.broadcasted_iota(jnp.int32, (H, HD), 0)
        d_col = lax.broadcasted_iota(jnp.int32, (H, HD), 1)
        diag = (d_col & (H - 1)) == d_row
        x5 = jnp.concatenate(
            [x[:, c * 128:(c + 1) * 128] for c in range(NXC)]
            + [jnp.zeros((8 - NXC, 128), _F32)], axis=0).astype(_BF16)
        xr = _dot(x5, e0)
        end.tick(4)
        qa = jnp.zeros((H, D), _F32)
        for c in range(NXC):
            sc = jnp.where(diag, jnp.broadcast_to(xr[c:c + 1, :], (H, HD)), 0.0).astype(_BF16)
            qa = qa + _dot(sc, wqa_v[pl.ds(c * HD, HD), :])
            end.tick(3)
        qa = (qa * scale).astype(_BF16)

        end.adv_to(p_up)
        qabs = []
        for b in range(NCB):
            t = _dot_nt(qa, wuk_v[pl.ds(b * HD, HD), :])
            mb = jnp.where(diag, t, 0.0).astype(_BF16)
            end.tick(4)
            qabs.append(_dot_nt(mb, e0))
            end.tick(4)
        qabs = jnp.concatenate(qabs, axis=1).astype(_BF16)

        end.adv_to(p_lat)
        KB = Sk // 4
        s = []
        for kb in range(4):
            s.append(_dot_nt(qabs, ckv_v[pl.ds(kb * KB, KB), :]))
            end.tick(3)
        s = jnp.concatenate(s, axis=1)
        m = jnp.max(s, axis=-1, keepdims=True)
        p = jnp.exp(s - m)
        l = jnp.sum(p, axis=-1, keepdims=True)
        p = p.astype(_BF16)
        end.tick(3)
        cl = jnp.zeros((H, Dc), _F32)
        for kb in range(4):
            cl = cl + _dot(p[:, kb * KB:(kb + 1) * KB], ckv_v[pl.ds(kb * KB, KB), :])
            end.tick(3)
        cl = (cl / l).astype(_BF16)

        ctx = jnp.zeros((H, D), _F32)
        for b in range(NCB):
            xb = _dot(cl[:, b * 128:(b + 1) * 128], e0)
            sb = jnp.where(diag, xb, 0.0).astype(_BF16)
            ctx = ctx + _dot(sb, wuv_v[pl.ds(b * HD, HD), :])
            end.tick(4)

        sub = lax.broadcasted_iota(jnp.int32, (8, D), 0)
        ctx = ctx * g
        lhs_a = jnp.concatenate(
            [jnp.where(sub == (h % 8), ctx[8 * (h // 8):8 * (h // 8) + 8, :], 0.0) for h in range(H)],
            axis=1).astype(_BF16)
        one_g = 1.0 - g
        lhs_b = jnp.concatenate(
            [jnp.where(sub == (h % 8), ob_s[h] * one_g, 0.0) for h in range(H)],
            axis=1).astype(_BF16)

        acc = jnp.zeros((8, M), _F32)
        o = 0
        target = p_lat
        for gi, (n, gr) in enumerate(zip(WO_GROUPS, wo_groups)):
            if gi < NPACED:
                target += len(gr)
                end.adv_to(target)
            else:
                for which, (us, buf) in enumerate(((u_woa, woa_v), (u_wob, wob_v))):
                    mine = in_grp(us, gi)
                    rows = buf.at[pl.ds(mine[0].row0, mine[-1].row1 - mine[0].row0)]
                    pltpu.make_async_copy(rows, rows, sem_f.at[which, gi - NPACED]).wait()
            acc = acc + _dot(lhs_a[:, o:o + n], woa_v[pl.ds(o, n), :])
            acc = acc + _dot(lhs_b[:, o:o + n], wob_v[pl.ds(o, n), :])
            o += n
        assert end.pos == end.lim
        o_ref[0] = jnp.sum(acc, axis=0, keepdims=True).astype(o_ref.dtype)

    any_spec = pl.BlockSpec(memory_space=pl.ANY)
    scratch = [
        pltpu.VMEM((1, 1, M), _BF16),
        pltpu.VMEM((M,), _BF16),
        pltpu.VMEM((M, HD), _BF16),
        pltpu.VMEM((NBUF, Sk, D), _BF16),
        pltpu.VMEM((NBUF, Sk, D), _BF16),
        pltpu.VMEM((M * H, D), _BF16),
        pltpu.VMEM((Dc * H, D), _BF16),
        pltpu.VMEM((Sk, Dc), _BF16),
        pltpu.VMEM((Dc * H, D), _BF16),
        pltpu.VMEM((HD, M), _BF16),
        pltpu.VMEM((HD, M), _BF16),
        pltpu.VMEM((H, 8, D), _F32),
        pltpu.VMEM((H, 8, D), _F32),
        pltpu.SemaphoreType.DMA((2, 4)),
        pltpu.SemaphoreType.DMA((2, NBUF)),
        pltpu.SemaphoreType.DMA((2, NBUF)),
        pltpu.SemaphoreType.DMA((2, NPACED)),
        pltpu.SemaphoreType.DMA((2, NEXACT)),
    ]
    return pl.pallas_call(
        kernel,
        out_shape=jax.ShapeDtypeStruct((B, Sq, M), A_x.dtype),
        in_specs=[any_spec] * 11,
        out_specs=pl.BlockSpec(memory_space=pltpu.VMEM),
        scratch_shapes=scratch,
        compiler_params=pltpu.CompilerParams(
            vmem_limit_bytes=100 * 1024 * 1024,
            disable_semaphore_checks=True, disable_bounds_checks=True),
    )(A_x, gate_w, B_wq, B_k_cache, B_v_cache, w_q2, w_uk2, A_c_kv, w_uv2, w_o2, B_wo)
```
